```python
import jax
import jax.numpy as jnp

def _softmax(x, axis=-1):
    return jax.nn.softmax(x, axis=axis)
def _gelu(x):
    return jax.nn.gelu(x, approximate=True)
def _silu(x):
    return jax.nn.silu(x)
def _sigmoid(x):
    return jax.nn.sigmoid(x)
def _layernorm(x, axis=-1, eps=1e-5):
    m = jnp.mean(x, axis=axis, keepdims=True)
    v = jnp.var(x, axis=axis, keepdims=True)
    return (x - m) / jnp.sqrt(v + eps)
def _scatter_add(tgt, idx, src, axis=0):
    return tgt.at[idx].add(src)
def _segment_sum(src, seg, n):
    return jax.ops.segment_sum(src, seg, n)
class _Rng:
    def __init__(self, key):
        self._k = key
    def _next(self):
        self._k, sub = jax.random.split(self._k)
        return sub
    def normal(self, shape):
        return jax.random.normal(self._next(), shape, dtype=jnp.bfloat16)
    def randint(self, lo, hi, shape):
        return jax.random.randint(self._next(), shape, lo, hi, dtype=jnp.int32)
    def uniform(self, shape, lo=0.0, hi=1.0):
        return jax.random.uniform(self._next(), shape, jnp.bfloat16, lo, hi)
    def permutation(self, n):
        return jax.random.permutation(self._next(), n)


kernel_name = 'gated_mix__compressed_kv_cla__gqa_block_cached__decode'

def setup_inputs():
    _rng = _Rng(jax.random.key(int.from_bytes(__import__("os").urandom(4), "little")))
    _w = (lambda a: (lambda t: t.astype(jnp.bfloat16) if jnp.issubdtype(t.dtype, jnp.floating) else t)(jnp.asarray(a)))
    def _A_setup():
        B, H, Sq, Sk, D, M = 1, 32, 1, 4096, 128, 640
        Dc = 4 * D
        return {
            "x": _w((lambda *s: _rng.normal(s) * 0.05)(B, Sq, M)),
            "c_kv": _w((lambda *s: _rng.normal(s) * 0.05)(B, Sk, Dc)),
            "w_q": _w((lambda *s: _rng.normal(s) * 0.05)(M, H, D) * (M ** -0.5)),
            "w_uk": _w((lambda *s: _rng.normal(s) * 0.05)(Dc, H, D) * (Dc ** -0.5)),
            "w_uv": _w((lambda *s: _rng.normal(s) * 0.05)(Dc, H, D) * (Dc ** -0.5)),
            "w_o": _w((lambda *s: _rng.normal(s) * 0.05)(H, D, M) * ((H * D) ** -0.5)),
        }
    _A_in = _A_setup()

    def _B_setup():
        B, Sq, D = 1, 1, 640
        Hq, Hkv, Sk, Dh = 32, 32, 4096, 128
        assert Hq % Hkv == 0, (Hq, Hkv)
        return {
            "x": _w((lambda *s: _rng.normal(s) * 0.05)(B, Sq, D)),
            "k_cache": _w((lambda *s: _rng.normal(s) * 0.05)(B, Hkv, Sk, Dh)),
            "v_cache": _w((lambda *s: _rng.normal(s) * 0.05)(B, Hkv, Sk, Dh)),
            "wq": _w((lambda *s: _rng.normal(s) * 0.05)(D, Hq * Dh) * (D ** -0.5)),
            "wo": _w((lambda *s: _rng.normal(s) * 0.05)(Hq * Dh, D) * ((Hq * Dh) ** -0.5)),
        }
    _B_in = _B_setup()

    return {
        "A_x": _A_in["x"],
        "A_c_kv": _A_in["c_kv"],
        "A_w_q": _A_in["w_q"],
        "A_w_uk": _A_in["w_uk"],
        "A_w_uv": _A_in["w_uv"],
        "A_w_o": _A_in["w_o"],
        "B_x": _B_in["x"],
        "B_k_cache": _B_in["k_cache"],
        "B_v_cache": _B_in["v_cache"],
        "B_wq": _B_in["wq"],
        "B_wo": _B_in["wo"],
        "gate_w": _w((lambda *s: _rng.normal(s) * 0.05)(640)),
    }

def reference(A_x, A_c_kv, A_w_q, A_w_uk, A_w_uv, A_w_o, B_x, B_k_cache, B_v_cache, B_wq, B_wo, gate_w):
    def _A_ref(x, c_kv, w_q, w_uk, w_uv, w_o):
        B, Sq, M = x.shape[0], x.shape[1], x.shape[2]
        Sk = c_kv.shape[1]
        H, D = w_q.shape[1], w_q.shape[2]
        q = jnp.einsum("bqm,mhd->bhqd", x, w_q)
        k = jnp.einsum("bkc,chd->bhkd", c_kv, w_uk)
        v = jnp.einsum("bkc,chd->bhkd", c_kv, w_uv)
        scores = jnp.einsum("bhqd,bhkd->bhqk", q, k) * (D ** -0.5)
        off = Sk - Sq
        qi = jnp.arange(Sq)[:, None]
        kj = jnp.arange(Sk)[None, :]
        cmask = kj <= (qi + off)
        scores = jnp.where(cmask[None, None], scores, -1e9)
        p = _softmax(scores, axis=-1)
        ctx = jnp.einsum("bhqk,bhkd->bhqd", p, v)
        return jnp.einsum("bhqd,hdm->bqm", ctx, w_o)

    def _B_ref(x, k_cache, v_cache, wq, wo):
        B, Sq, D = x.shape
        Hq, Dh = 32, 128
        Hkv = k_cache.shape[1]
        rep = Hq // Hkv
        q = (lambda x, *d: x.transpose(*d))((x @ wq).reshape(B, Sq, Hq, Dh), 0, 2, 1, 3)
        k = jnp.repeat(k_cache, rep, axis=1)
        v = jnp.repeat(v_cache, rep, axis=1)
        scores = jnp.einsum("bhqd,bhkd->bhqk", q, k) * (Dh ** -0.5)
        p = _softmax(scores, axis=-1)
        o = jnp.einsum("bhqk,bhkd->bhqd", p, v)
        return (lambda x, *d: x.transpose(*d))(o, 0, 2, 1, 3).reshape(B, Sq, Hq * Dh) @ wo

    x = A_x
    g = _sigmoid((x * gate_w).sum(-1, keepdims=True))
    a = _A_ref(x, A_c_kv, A_w_q, A_w_uk, A_w_uv, A_w_o)
    b = _B_ref(x, B_k_cache, B_v_cache, B_wq, B_wo)
    return g * a + (1 - g) * b
```

```python
import jax
import jax.numpy as jnp
import jax.experimental.pallas as pl
import jax.experimental.pallas.tpu as pltpu

H = 32
D = 128
S = 4096
M = 640
C = 512
BF = jnp.bfloat16
F32 = jnp.float32

LOOK = 4
RING = LOOK + 1
WIN = 8
WOB_CHUNKS = (1024, 1024, 1024, 512, 256, 128, 128)
WOA_CHUNKS = (1024, 1024, 1024, 1024)

_NT = (((1,), (1,)), ((), ()))


def _dot(a, b):
    return jnp.dot(a, b, preferred_element_type=F32)


def _dot_nt(a, b):
    return jax.lax.dot_general(a, b, _NT, preferred_element_type=F32)


def _kernel(x_hbm, gate_hbm, wqa_hbm, wuk_hbm, ckv_hbm, wuv_hbm, woa_hbm,
            wqb_hbm, k_hbm, v_hbm, wob_hbm,
            out_ref,
            x_v, gate_v, wqa_v, wuk_v, ckv_v, wuv_v, woa_v, wqb_v, wob_v,
            k_v, v_v, e_v, qb_v, ob_v,
            sem_s, sem_k, sem_v, sem_o):
    chunks = []

    def add(src, dst):
        chunks.append((src, dst))
        return len(chunks) - 1

    i_x = add(x_hbm, x_v)
    i_g = add(gate_hbm, gate_v)
    i_wqa = [add(wqa_hbm.at[pl.ds(b * 4096, 4096)], wqa_v.at[pl.ds(b * 4096, 4096)]) for b in range(5)]
    i_wuk = [add(wuk_hbm.at[pl.ds(b * 4096, 4096)], wuk_v.at[pl.ds(b * 4096, 4096)]) for b in range(4)]
    i_ckv = [add(ckv_hbm.at[pl.ds(b * 1024, 1024)], ckv_v.at[pl.ds(b * 1024, 1024)]) for b in range(4)]
    i_wuv = [add(wuv_hbm.at[pl.ds(b * 4096, 4096)], wuv_v.at[pl.ds(b * 4096, 4096)]) for b in range(4)]
    i_woa = []
    r = 0
    for n in WOA_CHUNKS:
        i_woa.append(add(woa_hbm.at[pl.ds(r, n)], woa_v.at[pl.ds(r, n)]))
        r += n
    i_wqb = [add(wqb_hbm.at[pl.ds(b * 128, 128)], wqb_v.at[pl.ds(b * 128, 128)]) for b in range(5)]
    n_static = len(chunks)

    def k_copy(h, slot):
        return pltpu.make_async_copy(k_hbm.at[h], k_v.at[slot], sem_k.at[slot])

    def v_copy(h, slot):
        return pltpu.make_async_copy(v_hbm.at[h], v_v.at[slot], sem_v.at[slot])

    def s_copy(i):
        return pltpu.make_async_copy(chunks[i][0], chunks[i][1], sem_s.at[i])

    order = [s_copy(i) for i in range(n_static)]
    for h in range(LOOK):
        order.append(k_copy(h, h))
        order.append(v_copy(h, h))
    state = {"next": 0}

    def issue_upto(n):
        n = min(n, len(order))
        while state["next"] < n:
            order[state["next"]].start()
            state["next"] += 1

    def wait_s(i):
        order[i].wait()
        issue_upto(i + 1 + WIN)

    issue_upto(2 + WIN)

    row = jax.lax.broadcasted_iota(jnp.int32, (128, 4096), 0)
    col = jax.lax.broadcasted_iota(jnp.int32, (128, 4096), 1)
    e_v[...] = jnp.where((col >> 5) == row, 1.0, 0.0).astype(BF)
    r32 = jax.lax.broadcasted_iota(jnp.int32, (H, 4096), 0)
    c32 = jax.lax.broadcasted_iota(jnp.int32, (H, 4096), 1)
    diag = (c32 & 31) == r32

    wait_s(i_x)
    wait_s(i_g)
    x = x_v[...]
    xf = x.astype(F32)
    gate = jax.nn.sigmoid(jnp.sum(xf * gate_v[...].astype(F32), axis=-1, keepdims=True))

    x5 = jnp.concatenate([x[:, b * 128:(b + 1) * 128] for b in range(5)]
                         + [jnp.zeros((3, 128), BF)], axis=0)
    xe = _dot(x5, e_v[...])
    qa = jnp.zeros((H, D), F32)
    for b in range(5):
        wait_s(i_wqa[b])
        sb = jnp.where(diag, jnp.broadcast_to(xe[b:b + 1, :], (H, 4096)), 0.0).astype(BF)
        qa = qa + _dot(sb, wqa_v[pl.ds(b * 4096, 4096), :])
    qa = qa.astype(BF)

    qabs = []
    for b in range(4):
        wait_s(i_wuk[b])
        rt = _dot_nt(qa, wuk_v[pl.ds(b * 4096, 4096), :])
        rt = jnp.where(diag, rt, 0.0).astype(BF)
        qabs.append(_dot_nt(rt, e_v[...]).astype(BF))
    qabs = jnp.concatenate(qabs, axis=1)

    sc = []
    for b in range(4):
        wait_s(i_ckv[b])
        sc.append(_dot_nt(qabs, ckv_v[pl.ds(b * 1024, 1024), :]))
    sa = jnp.concatenate(sc, axis=1)
    scale = D ** -0.5
    ma = jnp.max(sa, axis=-1, keepdims=True)
    pa = jnp.exp((sa - ma) * scale)
    la = jnp.sum(pa, axis=-1, keepdims=True)
    cc = (_dot(pa.astype(BF), ckv_v[...]) / la).astype(BF)

    ctx = jnp.zeros((H, D), F32)
    for b in range(4):
        wait_s(i_wuv[b])
        ex = _dot(cc[:, b * 128:(b + 1) * 128], e_v[...])
        ex = jnp.where(diag, ex, 0.0).astype(BF)
        ctx = ctx + _dot(ex, wuv_v[pl.ds(b * 4096, 4096), :])
    ctx = ctx.astype(BF).astype(F32)
    ctx_flat = jnp.concatenate([ctx[h:h + 1, :] for h in range(H)], axis=1).astype(BF)

    oa = jnp.zeros((1, M), F32)
    r = 0
    for j, n in enumerate(WOA_CHUNKS):
        wait_s(i_woa[j])
        oa = oa + _dot(ctx_flat[:, r:r + n], woa_v[pl.ds(r, n), :])
        r += n

    qb = jnp.zeros((1, 4096), F32)
    for b in range(5):
        wait_s(i_wqb[b])
        qb = qb + _dot(x[:, b * 128:(b + 1) * 128], wqb_v[pl.ds(b * 128, 128), :])
    for h in range(H):
        qb_v[h] = qb[:, h * 128:(h + 1) * 128].astype(BF)
    issue_upto(len(order))

    wob_copies = []
    r = 0
    for j, n in enumerate(WOB_CHUNKS):
        wob_copies.append(pltpu.make_async_copy(
            wob_hbm.at[pl.ds(r, n)], wob_v.at[pl.ds(r, n)], sem_o.at[j]))
        r += n

    def head(h, carry):
        slot = h % RING
        nslot = (h + LOOK) % RING
        k_copy(h, slot).wait()

        @pl.when(h + LOOK < H)
        def _():
            k_copy(h + LOOK, nslot).start()

        @pl.when(h + LOOK == H)
        def _():
            for c in wob_copies:
                c.start()

        s = _dot_nt(qb_v[h], k_v[slot])
        m = jnp.max(s, axis=-1, keepdims=True)
        p = jnp.exp((s - m) * scale)
        l = jnp.sum(p, axis=-1, keepdims=True)
        v_copy(h, slot).wait()

        @pl.when(h + LOOK < H)
        def _():
            v_copy(h + LOOK, nslot).start()

        o = _dot(p.astype(BF), v_v[slot]) / l
        ob_v[h] = o.astype(BF)
        return carry

    jax.lax.fori_loop(0, H, head, 0)

    ob_flat = jnp.concatenate([ob_v[h] for h in range(H)], axis=1)
    ob = jnp.zeros((1, M), F32)
    r = 0
    for j, n in enumerate(WOB_CHUNKS):
        wob_copies[j].wait()
        ob = ob + _dot(ob_flat[:, r:r + n], wob_v[pl.ds(r, n), :])
        r += n

    res = gate * oa + (1.0 - gate) * ob
    out_ref[...] = res.astype(out_ref.dtype)


@jax.jit
def pallas_gated_mix__compressed_kv_cla__gqa_block_cached__decode_kernel(
    A_x, A_c_kv, A_w_q, A_w_uk, A_w_uv, A_w_o,
    B_x, B_k_cache, B_v_cache, B_wq, B_wo, gate_w,
):
    x = A_x.reshape(1, M)
    gate = gate_w.reshape(1, M)
    wqa = A_w_q.reshape(M * H, D)
    wuk = A_w_uk.reshape(C * H, D)
    wuv = A_w_uv.reshape(C * H, D)
    woa = A_w_o.reshape(H * D, M)
    ckv = A_c_kv.reshape(S, C)
    k = B_k_cache.reshape(H, S, D)
    v = B_v_cache.reshape(H, S, D)

    n_static = 2 + 5 + 4 + 4 + 4 + len(WOA_CHUNKS) + 5
    any_spec = pl.BlockSpec(memory_space=pl.ANY)
    out = pl.pallas_call(
        _kernel,
        in_specs=[any_spec] * 11,
        out_specs=pl.BlockSpec(memory_space=pltpu.VMEM),
        out_shape=jax.ShapeDtypeStruct((1, M), BF),
        scratch_shapes=[
            pltpu.VMEM((1, M), BF),
            pltpu.VMEM((1, M), BF),
            pltpu.VMEM((M * H, D), BF),
            pltpu.VMEM((C * H, D), BF),
            pltpu.VMEM((S, C), BF),
            pltpu.VMEM((C * H, D), BF),
            pltpu.VMEM((H * D, M), BF),
            pltpu.VMEM((M, H * D), BF),
            pltpu.VMEM((H * D, M), BF),
            pltpu.VMEM((RING, S, D), BF),
            pltpu.VMEM((RING, S, D), BF),
            pltpu.VMEM((128, 4096), BF),
            pltpu.VMEM((H, 1, D), BF),
            pltpu.VMEM((H, 1, D), BF),
            pltpu.SemaphoreType.DMA((n_static,)),
            pltpu.SemaphoreType.DMA((RING,)),
            pltpu.SemaphoreType.DMA((RING,)),
            pltpu.SemaphoreType.DMA((len(WOB_CHUNKS),)),
        ],
        compiler_params=pltpu.CompilerParams(vmem_limit_bytes=100 * 1024 * 1024),
    )(x, gate, wqa, wuk, ckv, wuv, woa, B_wq, k, v, B_wo)
    return out.reshape(1, 1, M)
```

```python
import jax
import jax.numpy as jnp
import jax.experimental.pallas as pl
import jax.experimental.pallas.tpu as pltpu

H = 32
D = 128
S = 4096
M = 640
C = 512
BF = jnp.bfloat16
F32 = jnp.float32

CH = 256
NCH = S // CH
LO = 1
HI = 0
WIN = 8
WOA_CHUNKS = (1024, 1024, 1024, 1024)
WL = 16
WX = 3
WO_GROUPS = (4, 4, 4, 4, 4, 4, 4, 2, 1, 1)
PV_AT = 4

_NT = (((1,), (1,)), ((), ()))


def _dot(a, b):
    return jnp.dot(a, b, preferred_element_type=F32)


def _dot_nt(a, b):
    return jax.lax.dot_general(a, b, _NT, preferred_element_type=F32)


def _kernel(x_hbm, gate_hbm, wqa_hbm, wuk_hbm, ckv_hbm, wuv_hbm, woa_hbm,
            wqb_hbm, k_hbm, v_hbm, wob_hbm,
            out_ref,
            x_v, gate_v, wqa_v, wuk_v, ckv_v, wuv_v, woa_v, wqb_v, wob_v,
            k_v, v_v, e_v, qb_v, ob_v, s_v, p_v, l_v,
            sem_k, sem_v, sem_h):
    chunks = []

    def add(src, dst):
        chunks.append((src, dst))
        return len(chunks) - 1

    i_x = add(x_hbm, x_v)
    i_g = add(gate_hbm, gate_v)
    i_wqa = [add(wqa_hbm.at[pl.ds(b * 4096, 4096)], wqa_v.at[pl.ds(b * 4096, 4096)]) for b in range(5)]
    i_wuk = [add(wuk_hbm.at[pl.ds(b * 4096, 4096)], wuk_v.at[pl.ds(b * 4096, 4096)]) for b in range(4)]
    i_ckv = [add(ckv_hbm.at[pl.ds(b * 1024, 1024)], ckv_v.at[pl.ds(b * 1024, 1024)]) for b in range(4)]
    i_wuv = [add(wuv_hbm.at[pl.ds(b * 4096, 4096)], wuv_v.at[pl.ds(b * 4096, 4096)]) for b in range(4)]
    i_woa = []
    r = 0
    for n in WOA_CHUNKS:
        i_woa.append(add(woa_hbm.at[pl.ds(r, n)], woa_v.at[pl.ds(r, n)]))
        r += n
    i_wqb = [add(wqb_hbm.at[pl.ds(b * 128, 128)], wqb_v.at[pl.ds(b * 128, 128)]) for b in range(5)]
    n_static = len(chunks)

    def k_copy(h, slot, j):
        return pltpu.make_async_copy(k_hbm.at[h, pl.ds(j * CH, CH)], k_v.at[slot, pl.ds(j * CH, CH)],
                                     sem_k.at[j])

    def v_copy(h, slot, j):
        return pltpu.make_async_copy(v_hbm.at[h, pl.ds(j * CH, CH)], v_v.at[slot, pl.ds(j * CH, CH)],
                                     sem_v.at[j])

    def wol_copy(i):
        return pltpu.make_async_copy(wob_hbm.at[pl.ds(i * 128, 64)], wob_v.at[pl.ds(i * 128, 64)],
                                     sem_k.at[i % NCH])

    NH_SEM = WX + 5

    def woh_copy(i):
        return pltpu.make_async_copy(wob_hbm.at[pl.ds(i * 128 + 64, 64)], wob_v.at[pl.ds(i * 128 + 64, 64)],
                                     sem_h.at[i % NH_SEM])

    def s_copy(i):
        return pltpu.make_async_copy(chunks[i][0], chunks[i][1], sem_v.at[i % NCH])

    order = [s_copy(i) for i in range(n_static)]
    state = {"next": 0}

    def issue_upto(n):
        n = min(n, len(order))
        while state["next"] < n:
            order[state["next"]].start(priority=LO)
            state["next"] += 1

    def wait_s(i):
        order[i].wait()
        issue_upto(i + 1 + WIN)

    issue_upto(2 + WIN)

    row = jax.lax.broadcasted_iota(jnp.int32, (128, 4096), 0)
    col = jax.lax.broadcasted_iota(jnp.int32, (128, 4096), 1)
    e_v[...] = jnp.where((col >> 5) == row, 1.0, 0.0).astype(BF)
    r32 = jax.lax.broadcasted_iota(jnp.int32, (H, 4096), 0)
    c32 = jax.lax.broadcasted_iota(jnp.int32, (H, 4096), 1)
    diag = (c32 & 31) == r32

    wait_s(i_x)
    wait_s(i_g)
    x = x_v[...]
    xf = x.astype(F32)
    gate = jax.nn.sigmoid(jnp.sum(xf * gate_v[...].astype(F32).reshape(1, M), axis=-1, keepdims=True))

    x5 = jnp.concatenate([x[:, b * 128:(b + 1) * 128] for b in range(5)]
                         + [jnp.zeros((3, 128), BF)], axis=0)
    xe = _dot(x5, e_v[...])
    qa = jnp.zeros((H, D), F32)
    for b in range(5):
        wait_s(i_wqa[b])
        sb = jnp.where(diag, jnp.broadcast_to(xe[b:b + 1, :], (H, 4096)), 0.0).astype(BF)
        qa = qa + _dot(sb, wqa_v[pl.ds(b * 4096, 4096), :])
    qa = qa.astype(BF)

    qabs = []
    for b in range(4):
        wait_s(i_wuk[b])
        rt = _dot_nt(qa, wuk_v[pl.ds(b * 4096, 4096), :])
        rt = jnp.where(diag, rt, 0.0).astype(BF)
        qabs.append(_dot_nt(rt, e_v[...]).astype(BF))
    qabs = jnp.concatenate(qabs, axis=1)

    sc = []
    for b in range(4):
        wait_s(i_ckv[b])
        sc.append(_dot_nt(qabs, ckv_v[pl.ds(b * 1024, 1024), :]))
    sa = jnp.concatenate(sc, axis=1)
    scale = D ** -0.5
    ma = jnp.max(sa, axis=-1, keepdims=True)
    pa = jnp.exp((sa - ma) * scale)
    la = jnp.sum(pa, axis=-1, keepdims=True)
    cc = (_dot(pa.astype(BF), ckv_v[...]) / la).astype(BF)

    ctx = jnp.zeros((H, D), F32)
    for b in range(4):
        wait_s(i_wuv[b])
        ex = _dot(cc[:, b * 128:(b + 1) * 128], e_v[...])
        ex = jnp.where(diag, ex, 0.0).astype(BF)
        ctx = ctx + _dot(ex, wuv_v[pl.ds(b * 4096, 4096), :])
    ctx = ctx.astype(BF).astype(F32)
    ctx_flat = jnp.concatenate([ctx[h:h + 1, :] for h in range(H)], axis=1).astype(BF)

    oa = jnp.zeros((1, M), F32)
    r = 0
    for j, n in enumerate(WOA_CHUNKS):
        wait_s(i_woa[j])
        oa = oa + _dot(ctx_flat[:, r:r + n], woa_v[pl.ds(r, n), :])
        r += n

    qb = jnp.zeros((1, 4096), F32)
    for b in range(5):
        wait_s(i_wqb[b])
        for j in range(NCH):
            if j * 5 // NCH == b:
                k_copy(0, 0, j).start(priority=LO)
        qb = qb + _dot(x[:, b * 128:(b + 1) * 128], wqb_v[pl.ds(b * 128, 128), :])
    for h in range(H):
        qb_v[h] = qb[:, h * 128:(h + 1) * 128].astype(BF)

    scale = D ** -0.5

    def steps(h, do_pv, last):
        slot = h % 2
        pslot = 1 - slot
        q = qb_v[h]
        acc = jnp.zeros((1, D), F32)
        for j in range(NCH):
            k_copy(h, slot, j).wait()
            if do_pv:
                v_copy(h - 1, pslot, j).wait()
            if not last:
                k_copy(h + 1, pslot, j).start(priority=LO)
            else:
                wol_copy(j).start(priority=LO)
            v_copy(h, slot, j).start(priority=HI)
            s_v[:, j * CH:(j + 1) * CH] = _dot_nt(q, k_v[slot, pl.ds(j * CH, CH), :])
            if do_pv:
                acc = acc + _dot(p_v[:, j * CH:(j + 1) * CH], v_v[pslot, pl.ds(j * CH, CH), :])
        if do_pv:
            ob_v[h - 1] = (acc / l_v[...]).astype(BF)
        s = s_v[...]
        m = jnp.max(s, axis=-1, keepdims=True)
        p = jnp.exp((s - m) * scale)
        l_v[...] = jnp.broadcast_to(jnp.sum(p, axis=-1, keepdims=True), (1, D))
        p_v[...] = p.astype(BF)

    steps(0, False, False)

    def head(h, carry):
        steps(h, True, False)
        return carry

    jax.lax.fori_loop(1, H - 1, head, 0)
    steps(H - 1, True, True)

    for i in range(WX):
        woh_copy(i).start(priority=HI)
    ob = jnp.zeros((1, M), F32)
    pslot = (H - 1) % 2
    i = 0
    for g in WO_GROUPS:
        i0 = i
        for _ in range(g):
            wol_copy(i).wait()
            if i + WL < H:
                wol_copy(i + WL).start(priority=LO)
            if i + WX < H:
                woh_copy(i + WX).start(priority=HI)
            i += 1
        for ii in range(i0, i):
            woh_copy(ii).wait()
        if i0 <= PV_AT < i:
            for j in range(NCH):
                v_copy(H - 1, pslot, j).wait()
            ob_v[H - 1] = (_dot(p_v[...], v_v[pslot]) / l_v[...]).astype(BF)
        of = jnp.concatenate([ob_v[hh] for hh in range(i0, i)], axis=1) if g > 1 else ob_v[i0]
        ob = ob + _dot(of, wob_v[pl.ds(i0 * 128, g * 128), :])

    res = gate * oa + (1.0 - gate) * ob
    out_ref[...] = res.astype(out_ref.dtype)


@jax.jit
def pallas_gated_mix__compressed_kv_cla__gqa_block_cached__decode_kernel(
    A_x, A_c_kv, A_w_q, A_w_uk, A_w_uv, A_w_o,
    B_x, B_k_cache, B_v_cache, B_wq, B_wo, gate_w,
):
    x = A_x.reshape(1, M)
    wqa = A_w_q.reshape(M * H, D)
    wuk = A_w_uk.reshape(C * H, D)
    wuv = A_w_uv.reshape(C * H, D)
    woa = A_w_o.reshape(H * D, M)
    ckv = A_c_kv.reshape(S, C)
    k = B_k_cache.reshape(H, S, D)
    v = B_v_cache.reshape(H, S, D)

    any_spec = pl.BlockSpec(memory_space=pl.ANY)
    out = pl.pallas_call(
        _kernel,
        in_specs=[any_spec] * 11,
        out_specs=pl.BlockSpec(memory_space=pltpu.VMEM),
        out_shape=jax.ShapeDtypeStruct((1, M), BF),
        scratch_shapes=[
            pltpu.VMEM((1, M), BF),
            pltpu.VMEM((M,), BF),
            pltpu.VMEM((M * H, D), BF),
            pltpu.VMEM((C * H, D), BF),
            pltpu.VMEM((S, C), BF),
            pltpu.VMEM((C * H, D), BF),
            pltpu.VMEM((H * D, M), BF),
            pltpu.VMEM((M, H * D), BF),
            pltpu.VMEM((H * D, M), BF),
            pltpu.VMEM((2, S, D), BF),
            pltpu.VMEM((2, S, D), BF),
            pltpu.VMEM((128, 4096), BF),
            pltpu.VMEM((H, 1, D), BF),
            pltpu.VMEM((H, 1, D), BF),
            pltpu.VMEM((1, S), F32),
            pltpu.VMEM((1, S), BF),
            pltpu.VMEM((1, D), F32),
            pltpu.SemaphoreType.DMA((NCH,)),
            pltpu.SemaphoreType.DMA((NCH,)),
            pltpu.SemaphoreType.DMA((WX + 5,)),
        ],
        compiler_params=pltpu.CompilerParams(
            vmem_limit_bytes=100 * 1024 * 1024,
            disable_bounds_checks=True,
            disable_semaphore_checks=True),
    )(x, gate_w, wqa, wuk, ckv, wuv, woa, B_wq, k, v, B_wo)
    return out.reshape(1, 1, M)
```

```python
import jax
import jax.numpy as jnp
import jax.experimental.pallas as pl
import jax.experimental.pallas.tpu as pltpu

H = 32
D = 128
S = 4096
M = 640
C = 512
BF = jnp.bfloat16
F32 = jnp.float32

CH = 256
NCH = S // CH
LO = 1
HI = 0
HW = 8
WX = 3
WO_GROUPS = (4, 4, 4, 4, 4, 4, 4, 2, 2)
PV_AT = 2
BUDGET = 100
SCALE = D ** -0.5

_NT = (((1,), (1,)), ((), ()))


def _dot(a, b):
    return jnp.dot(a, b, preferred_element_type=F32)


def _dot_nt(a, b):
    return jax.lax.dot_general(a, b, _NT, preferred_element_type=F32)


def _diag(n):
    r = jax.lax.broadcasted_iota(jnp.int32, (H, n), 0)
    c = jax.lax.broadcasted_iota(jnp.int32, (H, n), 1)
    return (c & 31) == r


def _kernel(x_hbm, gate_hbm, wqa_hbm, wuk_hbm, ckv_hbm, wuv_hbm, woa_hbm,
            wqb_hbm, k_hbm, v_hbm, wob_hbm,
            out_ref,
            x_v, gate_v, wqa_v, wuk_v, ckv_v, wuv_v, woa_v, wqb_v, wob_v,
            k_v, v_v, e_v, qb_v, ob_v, s_v, p_v, l_v,
            xe_v, rt_v, sa_v, cc_v, ex_v, qacc_v,
            sem_k, sem_v, sem_h):
    lo_list, hi_list = [], []

    def add(lst, src, dst, rows):
        n = src.shape[0] // rows
        t0 = len(lst)
        for i in range(n):
            lst.append((src.at[pl.ds(i * rows, rows)], dst.at[pl.ds(i * rows, rows)]))
        return t0

    t_q = add(lo_list, wqa_hbm, wqa_v, 256)
    t_c = add(lo_list, ckv_hbm, ckv_v, 64)
    t_o = add(lo_list, woa_hbm, woa_v, 64)
    t_u = add(hi_list, wuk_hbm, wuk_v, 256)
    t_v = add(hi_list, wuv_hbm, wuv_v, 256)
    t_w = add(hi_list, wqb_hbm, wqb_v, 8)
    n_st = len(lo_list)
    assert n_st == len(hi_list) and n_st % NCH == 0

    def lo_copy(t):
        return pltpu.make_async_copy(lo_list[t][0], lo_list[t][1], sem_k.at[t % NCH])

    def hi_copy(t):
        return pltpu.make_async_copy(hi_list[t][0], hi_list[t][1], sem_v.at[t % NCH])

    def k_copy(h, slot, j):
        return pltpu.make_async_copy(k_hbm.at[h, pl.ds(j * CH, CH)], k_v.at[slot, pl.ds(j * CH, CH)],
                                     sem_k.at[j])

    def v_copy(h, slot, j):
        return pltpu.make_async_copy(v_hbm.at[h, pl.ds(j * CH, CH)], v_v.at[slot, pl.ds(j * CH, CH)],
                                     sem_v.at[j])

    def wol_copy(i):
        return pltpu.make_async_copy(wob_hbm.at[pl.ds(i * 64, 64)], wob_v.at[pl.ds(i * 64, 64)],
                                     sem_k.at[i % NCH])

    NH_SEM = WX + 5

    def woh_copy(i):
        return pltpu.make_async_copy(wob_hbm.at[pl.ds(2048 + i * 64, 64)], wob_v.at[pl.ds(2048 + i * 64, 64)],
                                     sem_h.at[i % NH_SEM])

    x_copy = pltpu.make_async_copy(x_hbm, x_v, sem_h.at[0])
    g_copy = pltpu.make_async_copy(gate_hbm, gate_v, sem_h.at[1])
    x_copy.start(priority=HI)
    g_copy.start(priority=HI)
    for t in range(NCH):
        lo_copy(t).start(priority=LO)
    for t in range(NCH):
        hi_copy(t).start(priority=HI)

    row = jax.lax.broadcasted_iota(jnp.int32, (128, 4096), 0)
    col = jax.lax.broadcasted_iota(jnp.int32, (128, 4096), 1)
    e_v[...] = jnp.where((col >> 5) == row, 1.0, 0.0).astype(BF)

    x_copy.wait()
    g_copy.wait()
    x = x_v[...]
    xf = x.astype(F32)
    gate = jax.nn.sigmoid(jnp.sum(xf * gate_v[...].astype(F32).reshape(1, M), axis=-1, keepdims=True))
    x5 = jnp.concatenate([x[:, b * 128:(b + 1) * 128] for b in range(5)]
                         + [jnp.zeros((3, 128), BF)], axis=0)
    xe = _dot(x5, e_v[...])
    xe_v[...] = xe

    st = {}

    def q_item(i):
        def f():
            b, p = divmod(i, 8)
            xr = xe_v[b:b + 1, 512 * p:512 * (p + 1)]
            sb = jnp.where(_diag(512), jnp.broadcast_to(xr, (H, 512)), 0.0).astype(BF)
            r = _dot(sb, wqa_v[pl.ds(512 * i, 512), :])
            st["qa"] = r if i == 0 else st["qa"] + r
            if i == 39:
                st["qa"] = st["qa"].astype(BF)
        return f

    def u_item(i):
        def f():
            b, p = divmod(i, 8)
            rt = _dot_nt(st["qa"], wuk_v[pl.ds(512 * i, 512), :])
            rt_v[32 * b:32 * (b + 1), 512 * p:512 * (p + 1)] = jnp.where(_diag(512), rt, 0.0).astype(BF)
        return f

    def gu_item(k):
        def f():
            r = _dot_nt(rt_v[:, 1024 * k:1024 * (k + 1)], e_v[:, 1024 * k:1024 * (k + 1)])
            st["qs"] = r if k == 0 else st["qs"] + r
            if k == 3:
                qs = st["qs"].astype(BF)
                st["qabs"] = jnp.concatenate([qs[32 * b:32 * (b + 1), :] for b in range(4)], axis=1)
        return f

    def c_item(i):
        def f():
            s = _dot_nt(st["qabs"], ckv_v[pl.ds(128 * i, 128), :])
            sa_v[:, 128 * i:128 * (i + 1)] = s
            st["mx"] = s if i == 0 else jnp.maximum(st["mx"], s)
            if i == 31:
                st["ma"] = jnp.max(st["mx"], axis=-1, keepdims=True)
        return f

    def pv_item(k):
        def f():
            p = jnp.exp((sa_v[:, 512 * k:512 * (k + 1)] - st["ma"]) * SCALE)
            ps = p[:, 0:128] + p[:, 128:256] + p[:, 256:384] + p[:, 384:512]
            st["ls"] = ps if k == 0 else st["ls"] + ps
            r = _dot(p.astype(BF), ckv_v[pl.ds(512 * k, 512), :])
            if k == 0:
                cc_v[...] = r
            elif k < 7:
                cc_v[...] = cc_v[...] + r
            else:
                la = jnp.sum(st["ls"], axis=-1, keepdims=True)
                cc = ((cc_v[...] + r) / la).astype(BF)
                st["cs"] = jnp.concatenate([cc[:, 128 * b:128 * (b + 1)] for b in range(4)], axis=0)
        return f

    def gv_item(k):
        def f():
            ex = _dot(st["cs"], e_v[:, 1024 * k:1024 * (k + 1)])
            r = jax.lax.broadcasted_iota(jnp.int32, (128, 1024), 0)
            c = jax.lax.broadcasted_iota(jnp.int32, (128, 1024), 1)
            ex_v[:, 1024 * k:1024 * (k + 1)] = jnp.where((c & 31) == (r & 31), ex, 0.0).astype(BF)
        return f

    def v_item(i):
        def f():
            b, p = divmod(i, 8)
            r = _dot(ex_v[32 * b:32 * (b + 1), 512 * p:512 * (p + 1)], wuv_v[pl.ds(512 * i, 512), :])
            st["ctx"] = r if i == 0 else st["ctx"] + r
            if i == 31:
                ctx = st["ctx"].astype(BF).astype(F32)
                st["cf"] = jnp.concatenate([ctx[h:h + 1, :] for h in range(H)], axis=1).astype(BF)
        return f

    def o_item(i):
        def f():
            r = _dot(st["cf"][:, 128 * i:128 * (i + 1)], woa_v[pl.ds(128 * i, 128), :])
            st["oa"] = r if i == 0 else st["oa"] + r
        return f

    def w_item(i):
        def f():
            b, p = divmod(i, 8)
            r = _dot(x[:, 128 * b:128 * (b + 1)], wqb_v[pl.ds(128 * b, 128), pl.ds(512 * p, 512)])
            if b == 0:
                qacc_v[:, 512 * p:512 * (p + 1)] = r
            elif b < 4:
                qacc_v[:, 512 * p:512 * (p + 1)] = qacc_v[:, 512 * p:512 * (p + 1)] + r
            else:
                qb = (qacc_v[:, 512 * p:512 * (p + 1)] + r).astype(BF)
                for hh in range(4):
                    qb_v[4 * p + hh] = qb[:, 128 * hh:128 * (hh + 1)]
        return f

    chain_a = []
    for i in range(40):
        chain_a.append((t_q + 2 * i + 1, 32, q_item(i), i == 39))
    for i in range(32):
        chain_a.append((t_u + 2 * i + 1 - HW, 64, u_item(i), i in (25, 27, 29, 31)))
        if i in (25, 27, 29, 31):
            chain_a.append((0, 128, gu_item((i - 25) // 2), i == 31))
    for i in range(32):
        chain_a.append((t_c + 2 * i + 1, 64, c_item(i), i == 31))
    for k in range(8):
        chain_a.append((0, 128, pv_item(k), k == 7))
    for k in range(4):
        chain_a.append((0, 128, gv_item(k), True if k == 3 else False))
    for i in range(32):
        chain_a.append((t_v + 2 * i + 1 - HW, 32, v_item(i), i == 31))
    for i in range(32):
        chain_a.append((t_o + 2 * i + 1, 40, o_item(i), False))
    chain_w = [(t_w + 16 * (i // 8) + 15 - HW, 32, w_item(i), False) for i in range(40)]

    for t in range(HW):
        hi_copy(t).wait()
    ia = iw = 0
    for t in range(n_st):
        lo_copy(t).wait()
        if t + HW < n_st:
            hi_copy(t + HW).wait()
        if t + NCH < n_st:
            lo_copy(t + NCH).start(priority=LO)
            hi_copy(t + NCH).start(priority=HI)
        else:
            k_copy(0, 0, t + NCH - n_st).start(priority=LO)
        used = 0
        last = t == n_st - 1
        while ia < len(chain_a) and chain_a[ia][0] <= t and (used + chain_a[ia][1] <= BUDGET or used == 0 or last):
            used += chain_a[ia][1]
            chain_a[ia][2]()
            fence = chain_a[ia][3]
            ia += 1
            if fence and not last:
                break
        while iw < len(chain_w) and chain_w[iw][0] <= t and (used + chain_w[iw][1] <= BUDGET or used == 0 or last):
            used += chain_w[iw][1]
            chain_w[iw][2]()
            iw += 1
    assert ia == len(chain_a) and iw == len(chain_w)
    oa = st["oa"]

    def steps(h, do_pv, last):
        slot = h % 2
        pslot = 1 - slot
        q = qb_v[h]
        acc = jnp.zeros((1, D), F32)
        for j in range(NCH):
            k_copy(h, slot, j).wait()
            if do_pv:
                v_copy(h - 1, pslot, j).wait()
            if not last:
                k_copy(h + 1, pslot, j).start(priority=LO)
            else:
                wol_copy(j).start(priority=LO)
            v_copy(h, slot, j).start(priority=HI)
            s_v[:, j * CH:(j + 1) * CH] = _dot_nt(q, k_v[slot, pl.ds(j * CH, CH), :])
            if do_pv:
                acc = acc + _dot(p_v[:, j * CH:(j + 1) * CH], v_v[pslot, pl.ds(j * CH, CH), :])
        if do_pv:
            ob_v[h - 1] = (acc / l_v[...]).astype(BF)
        s = s_v[...]
        m = jnp.max(s, axis=-1, keepdims=True)
        p = jnp.exp((s - m) * SCALE)
        l_v[...] = jnp.broadcast_to(jnp.sum(p, axis=-1, keepdims=True), (1, D))
        p_v[...] = p.astype(BF)

    steps(0, False, False)

    def head(h, carry):
        steps(h, True, False)
        return carry

    jax.lax.fori_loop(1, H - 1, head, 0)
    steps(H - 1, True, True)

    for i in range(WX):
        woh_copy(i).start(priority=HI)
    ob = jnp.zeros((1, M), F32)
    pslot = (H - 1) % 2
    i = 0
    for g in WO_GROUPS:
        i0 = i
        for _ in range(g):
            wol_copy(i).wait()
            if i + NCH < H:
                wol_copy(i + NCH).start(priority=LO)
            if i + WX < H:
                woh_copy(i + WX).start(priority=HI)
            i += 1
        for ii in range(i0, i):
            woh_copy(ii).wait()
        if i0 <= PV_AT < i:
            for j in range(NCH):
                v_copy(H - 1, pslot, j).wait()
            ob_v[H - 1] = (_dot(p_v[...], v_v[pslot]) / l_v[...]).astype(BF)
        h0, nh = i0 // 2, g // 2
        of_lo = jnp.concatenate([ob_v[hh] for hh in range(h0, h0 + nh)], axis=1) if nh > 1 else ob_v[h0]
        of_hi = jnp.concatenate([ob_v[16 + hh] for hh in range(h0, h0 + nh)], axis=1) if nh > 1 else ob_v[16 + h0]
        ob = ob + _dot(of_hi, wob_v[pl.ds(2048 + h0 * 128, nh * 128), :])
        ob = ob + _dot(of_lo, wob_v[pl.ds(h0 * 128, nh * 128), :])

    res = gate * oa + (1.0 - gate) * ob
    out_ref[...] = res.astype(out_ref.dtype)


@jax.jit
def pallas_gated_mix__compressed_kv_cla__gqa_block_cached__decode_kernel(
    A_x, A_c_kv, A_w_q, A_w_uk, A_w_uv, A_w_o,
    B_x, B_k_cache, B_v_cache, B_wq, B_wo, gate_w,
):
    x = A_x.reshape(1, M)
    wqa = A_w_q.reshape(M * H, D)
    wuk = A_w_uk.reshape(C * H, D)
    wuv = A_w_uv.reshape(C * H, D)
    woa = A_w_o.reshape(H * D, M)
    ckv = A_c_kv.reshape(S, C)
    k = B_k_cache.reshape(H, S, D)
    v = B_v_cache.reshape(H, S, D)

    any_spec = pl.BlockSpec(memory_space=pl.ANY)
    out = pl.pallas_call(
        _kernel,
        in_specs=[any_spec] * 11,
        out_specs=pl.BlockSpec(memory_space=pltpu.VMEM),
        out_shape=jax.ShapeDtypeStruct((1, M), BF),
        scratch_shapes=[
            pltpu.VMEM((1, M), BF),
            pltpu.VMEM((M,), BF),
            pltpu.VMEM((M * H, D), BF),
            pltpu.VMEM((C * H, D), BF),
            pltpu.VMEM((S, C), BF),
            pltpu.VMEM((C * H, D), BF),
            pltpu.VMEM((H * D, M), BF),
            pltpu.VMEM((M, H * D), BF),
            pltpu.VMEM((H * D, M), BF),
            pltpu.VMEM((2, S, D), BF),
            pltpu.VMEM((2, S, D), BF),
            pltpu.VMEM((128, 4096), BF),
            pltpu.VMEM((H, 1, D), BF),
            pltpu.VMEM((H, 1, D), BF),
            pltpu.VMEM((1, S), F32),
            pltpu.VMEM((1, S), BF),
            pltpu.VMEM((1, D), F32),
            pltpu.VMEM((8, 4096), F32),
            pltpu.VMEM((128, 4096), BF),
            pltpu.VMEM((H, S), F32),
            pltpu.VMEM((H, C), F32),
            pltpu.VMEM((128, 4096), BF),
            pltpu.VMEM((1, 4096), F32),
            pltpu.SemaphoreType.DMA((NCH,)),
            pltpu.SemaphoreType.DMA((NCH,)),
            pltpu.SemaphoreType.DMA((WX + 5,)),
        ],
        compiler_params=pltpu.CompilerParams(
            vmem_limit_bytes=100 * 1024 * 1024,
            disable_bounds_checks=True,
            disable_semaphore_checks=True),
    )(x, gate_w, wqa, wuk, ckv, wuv, woa, B_wq, k, v, B_wo)
    return out.reshape(1, 1, M)
```

```python
import jax
import jax.numpy as jnp
import jax.experimental.pallas as pl
import jax.experimental.pallas.tpu as pltpu

H = 32
D = 128
S = 4096
M = 640
C = 512
BF = jnp.bfloat16
F32 = jnp.float32

CH = 256
NCH = S // CH
LO = 1
HI = 0
HW = 8
WX = 10
BUDGET = 100
SCALE = D ** -0.5

_NT = (((1,), (1,)), ((), ()))


def _dot(a, b):
    return jnp.dot(a, b, preferred_element_type=F32)


def _dot_nt(a, b):
    return jax.lax.dot_general(a, b, _NT, preferred_element_type=F32)


def _diag(n):
    r = jax.lax.broadcasted_iota(jnp.int32, (H, n), 0)
    c = jax.lax.broadcasted_iota(jnp.int32, (H, n), 1)
    return (c & 31) == r


def _kernel(x_hbm, gate_hbm, wqa_hbm, wuk_hbm, ckv_hbm, wuv_hbm, woa_hbm,
            wqb_hbm, k_hbm, v_hbm, wob_hbm,
            out_ref,
            x_v, gate_v, wqa_v, wuk_v, ckv_v, wuv_v, woa_v, wqb_v, wob_v,
            k_v, v_v, e_v, qb_v, ob_v, s_v, p_v, l_v,
            xe_v, rt_v, sa_v, cc_v, ex_v, qacc_v,
            sem_k, sem_v, sem_h):
    lo_list, hi_list = [], []

    def add(lst, src, dst, rows):
        n = src.shape[0] // rows
        t0 = len(lst)
        for i in range(n):
            lst.append((src.at[pl.ds(i * rows, rows)], dst.at[pl.ds(i * rows, rows)]))
        return t0

    t_q = add(lo_list, wqa_hbm, wqa_v, 256)
    t_c = add(lo_list, ckv_hbm, ckv_v, 64)
    t_o = add(lo_list, woa_hbm, woa_v, 64)
    t_u = add(hi_list, wuk_hbm, wuk_v, 256)
    t_v = add(hi_list, wuv_hbm, wuv_v, 256)
    t_w = add(hi_list, wqb_hbm, wqb_v, 8)
    n_st = len(lo_list)
    assert n_st == len(hi_list) and n_st % NCH == 0

    def lo_copy(t):
        return pltpu.make_async_copy(lo_list[t][0], lo_list[t][1], sem_k.at[t % NCH])

    def hi_copy(t):
        return pltpu.make_async_copy(hi_list[t][0], hi_list[t][1], sem_v.at[t % NCH])

    def k_copy(h, slot, j):
        return pltpu.make_async_copy(k_hbm.at[h, pl.ds(j * CH, CH)], k_v.at[slot, pl.ds(j * CH, CH)],
                                     sem_k.at[j])

    def v_copy(h, slot, j):
        return pltpu.make_async_copy(v_hbm.at[h, pl.ds(j * CH, CH)], v_v.at[slot, pl.ds(j * CH, CH)],
                                     sem_v.at[j])

    def wol_copy(i):
        return pltpu.make_async_copy(wob_hbm.at[pl.ds(i * 64, 64)], wob_v.at[pl.ds(i * 64, 64)],
                                     sem_k.at[i % NCH])

    NH_SEM = WX + 5

    def woh_copy(i):
        return pltpu.make_async_copy(wob_hbm.at[pl.ds(2048 + i * 64, 64)], wob_v.at[pl.ds(2048 + i * 64, 64)],
                                     sem_h.at[i % NH_SEM])

    x_copy = pltpu.make_async_copy(x_hbm, x_v, sem_h.at[0])
    g_copy = pltpu.make_async_copy(gate_hbm, gate_v, sem_h.at[1])
    x_copy.start(priority=HI)
    g_copy.start(priority=HI)
    for t in range(NCH):
        lo_copy(t).start(priority=LO)
    for t in range(NCH):
        hi_copy(t).start(priority=HI)

    row = jax.lax.broadcasted_iota(jnp.int32, (128, 4096), 0)
    col = jax.lax.broadcasted_iota(jnp.int32, (128, 4096), 1)
    e_v[...] = jnp.where((col >> 5) == row, 1.0, 0.0).astype(BF)

    x_copy.wait()
    g_copy.wait()
    x = x_v[...]
    xf = x.astype(F32)
    gate = jax.nn.sigmoid(jnp.sum(xf * gate_v[...].astype(F32).reshape(1, M), axis=-1, keepdims=True))
    x5 = jnp.concatenate([x[:, b * 128:(b + 1) * 128] for b in range(5)]
                         + [jnp.zeros((3, 128), BF)], axis=0)
    xe = _dot(x5, e_v[...])
    xe_v[...] = xe

    st = {}

    QR = 256

    def q_item(i):
        def f():
            b, p = divmod(i, 4096 // QR)
            xr = xe_v[b:b + 1, QR * p:QR * (p + 1)]
            sb = jnp.where(_diag(QR), jnp.broadcast_to(xr, (H, QR)), 0.0).astype(BF)
            r = _dot(sb, wqa_v[pl.ds(QR * i, QR), :])
            st["qa"] = r if i == 0 else st["qa"] + r
            if i == 20480 // QR - 1:
                st["qa"] = st["qa"].astype(BF)
        return f

    def u_item(i):
        def f():
            b, p = divmod(i, 8)
            rt = _dot_nt(st["qa"], wuk_v[pl.ds(512 * i, 512), :])
            rt_v[32 * b:32 * (b + 1), 512 * p:512 * (p + 1)] = jnp.where(_diag(512), rt, 0.0).astype(BF)
        return f

    def gu_item(k):
        def f():
            r = _dot_nt(rt_v[:, 1024 * k:1024 * (k + 1)], e_v[:, 1024 * k:1024 * (k + 1)])
            st["qs"] = r if k == 0 else st["qs"] + r
            if k == 3:
                qs = st["qs"].astype(BF)
                st["qabs"] = jnp.concatenate([qs[32 * b:32 * (b + 1), :] for b in range(4)], axis=1)
        return f

    def c_item(i):
        def f():
            s = _dot_nt(st["qabs"], ckv_v[pl.ds(128 * i, 128), :])
            sa_v[:, 128 * i:128 * (i + 1)] = s
            st["mx"] = s if i == 0 else jnp.maximum(st["mx"], s)
            if i == 31:
                st["ma"] = jnp.max(st["mx"], axis=-1, keepdims=True)
        return f

    def pv_item(k):
        def f():
            p = jnp.exp((sa_v[:, 512 * k:512 * (k + 1)] - st["ma"]) * SCALE)
            ps = p[:, 0:128] + p[:, 128:256] + p[:, 256:384] + p[:, 384:512]
            st["ls"] = ps if k == 0 else st["ls"] + ps
            r = _dot(p.astype(BF), ckv_v[pl.ds(512 * k, 512), :])
            if k == 0:
                cc_v[...] = r
            elif k < 7:
                cc_v[...] = cc_v[...] + r
            else:
                la = jnp.sum(st["ls"], axis=-1, keepdims=True)
                cc = ((cc_v[...] + r) / la).astype(BF)
                st["cs"] = jnp.concatenate([cc[:, 128 * b:128 * (b + 1)] for b in range(4)], axis=0)
        return f

    def gv_item(k):
        def f():
            ex = _dot(st["cs"], e_v[:, 1024 * k:1024 * (k + 1)])
            r = jax.lax.broadcasted_iota(jnp.int32, (128, 1024), 0)
            c = jax.lax.broadcasted_iota(jnp.int32, (128, 1024), 1)
            ex_v[:, 1024 * k:1024 * (k + 1)] = jnp.where((c & 31) == (r & 31), ex, 0.0).astype(BF)
        return f

    def v_item(i):
        def f():
            b, p = divmod(i, 8)
            r = _dot(ex_v[32 * b:32 * (b + 1), 512 * p:512 * (p + 1)], wuv_v[pl.ds(512 * i, 512), :])
            st["ctx"] = r if i == 0 else st["ctx"] + r
            if i == 31:
                ctx = st["ctx"].astype(BF).astype(F32)
                st["cf"] = jnp.concatenate([ctx[h:h + 1, :] for h in range(H)], axis=1).astype(BF)
        return f

    def o_item(i):
        def f():
            r = _dot(st["cf"][:, 128 * i:128 * (i + 1)], woa_v[pl.ds(128 * i, 128), :])
            st["oa"] = r if i == 0 else st["oa"] + r
        return f

    def w_item(i):
        def f():
            b, p = divmod(i, 8)
            r = _dot(x[:, 128 * b:128 * (b + 1)], wqb_v[pl.ds(128 * b, 128), pl.ds(512 * p, 512)])
            if b == 0:
                qacc_v[:, 512 * p:512 * (p + 1)] = r
            elif b < 4:
                qacc_v[:, 512 * p:512 * (p + 1)] = qacc_v[:, 512 * p:512 * (p + 1)] + r
            else:
                qb = (qacc_v[:, 512 * p:512 * (p + 1)] + r).astype(BF)
                for hh in range(4):
                    qb_v[4 * p + hh] = qb[:, 128 * hh:128 * (hh + 1)]
        return f

    chain_a = []
    for i in range(20480 // QR):
        chain_a.append((t_q + (QR // 256) * (i + 1) - 1, 100 if QR == 256 else 32, q_item(i), i == 20480 // QR - 1))
    for i in range(32):
        chain_a.append((t_u + 2 * i + 1 - HW, 64, u_item(i), i in (25, 27, 29, 31)))
        if i in (25, 27, 29, 31):
            chain_a.append((0, 128, gu_item((i - 25) // 2), i == 31))
    for i in range(32):
        chain_a.append((t_c + 2 * i + 1, 64, c_item(i), i == 31))
    for k in range(8):
        chain_a.append((0, 128, pv_item(k), k == 7))
    for k in range(4):
        chain_a.append((0, 128, gv_item(k), True if k == 3 else False))
    for i in range(32):
        chain_a.append((t_v + 2 * i + 1 - HW, 32, v_item(i), i == 31))
    for i in range(32):
        chain_a.append((t_o + 2 * i + 1, 40, o_item(i), False))
    chain_w = [(t_w + 16 * (i // 8) + 15 - HW, 32, w_item(i), False) for i in range(40)]

    for t in range(HW):
        hi_copy(t).wait()
    ia = iw = 0
    for t in range(n_st):
        lo_copy(t).wait()
        if t + HW < n_st:
            hi_copy(t + HW).wait()
        if t + NCH < n_st:
            lo_copy(t + NCH).start(priority=LO)
            hi_copy(t + NCH).start(priority=HI)
        else:
            k_copy(0, 0, t + NCH - n_st).start(priority=LO)
        used = 0
        last = t == n_st - 1
        while ia < len(chain_a) and chain_a[ia][0] <= t and (used + chain_a[ia][1] <= BUDGET or used == 0 or last):
            used += chain_a[ia][1]
            chain_a[ia][2]()
            fence = chain_a[ia][3]
            ia += 1
            if fence and not last:
                break
        while iw < len(chain_w) and chain_w[iw][0] <= t and (used + chain_w[iw][1] <= BUDGET or used == 0 or last):
            used += chain_w[iw][1]
            chain_w[iw][2]()
            iw += 1
    assert ia == len(chain_a) and iw == len(chain_w)
    oa = st["oa"]

    def steps(h, do_pv, last):
        slot = h % 2
        pslot = 1 - slot
        q = qb_v[h]
        acc = jnp.zeros((1, D), F32)
        for j in range(NCH):
            k_copy(h, slot, j).wait()
            if do_pv:
                v_copy(h - 1, pslot, j).wait()
            if not last:
                k_copy(h + 1, pslot, j).start(priority=LO)
            else:
                wol_copy(j).start(priority=LO)
            v_copy(h, slot, j).start(priority=HI)
            s_v[:, j * CH:(j + 1) * CH] = _dot_nt(q, k_v[slot, pl.ds(j * CH, CH), :])
            if do_pv:
                acc = acc + _dot(p_v[:, j * CH:(j + 1) * CH], v_v[pslot, pl.ds(j * CH, CH), :])
        if do_pv:
            ob_v[h - 1] = (acc / l_v[...]).astype(BF)
        s = s_v[...]
        m = jnp.max(s, axis=-1, keepdims=True)
        p = jnp.exp((s - m) * SCALE)
        l_v[...] = jnp.broadcast_to(jnp.sum(p, axis=-1, keepdims=True), (1, D))
        p_v[...] = p.astype(BF)

    steps(0, False, False)

    def head(h, carry):
        steps(h, True, False)
        return carry

    jax.lax.fori_loop(1, H - 1, head, 0)
    steps(H - 1, True, True)

    for i in range(WX):
        woh_copy(i).start(priority=HI)
    ob = jnp.zeros((1, M), F32)
    pslot = (H - 1) % 2
    NV = 2
    GRP = 4
    lo_done = 0
    hi_done = 0
    hi_waited = 0
    acc8 = None
    for i in range(H):
        wol_copy(i).wait()
        if i + NCH < H:
            wol_copy(i + NCH).start(priority=LO)
        if i + WX < H:
            woh_copy(i + WX).start(priority=HI)
        if i >= H - NV:
            r0 = 64 * i
            w = wob_v[pl.ds(r0, 64), :].astype(F32)
            oc = obc[r0 - 15 * 128:r0 - 15 * 128 + 64, :]
            pr = w * jnp.concatenate([oc] * 5, axis=1)
            pr = pr.reshape(8, 8, M).sum(axis=0)
            acc8 = pr if acc8 is None else acc8 + pr
            continue
        boundary = (i + 1) % GRP == 0 or i == H - NV - 1
        if not boundary:
            continue
        if i == GRP - 1:
            for j in range(NCH):
                v_copy(H - 1, pslot, j).wait()
            ob_v[H - 1] = (_dot(p_v[...], v_v[pslot]) / l_v[...]).astype(BF)
            o15 = ob_v[15].astype(F32)
            obc = jnp.broadcast_to(o15, (128, 128)).T
        hi_avail = H if i == H - NV - 1 else min(H, i + 1 + 4)
        for ii in range(hi_waited, hi_avail):
            woh_copy(ii).wait()
        hi_waited = max(hi_waited, hi_avail)
        hi_heads = hi_waited // 2
        lo_heads = (i + 1) // 2
        if i == H - NV - 1 and NV < 2:
            raise NotImplementedError
        if lo_heads > lo_done:
            of = jnp.concatenate([ob_v[hh] for hh in range(lo_done, lo_heads)], axis=1)
            ob = ob + _dot(of, wob_v[pl.ds(lo_done * 128, (lo_heads - lo_done) * 128), :])
            lo_done = lo_heads
        if hi_heads > hi_done:
            of = jnp.concatenate([ob_v[16 + hh] for hh in range(hi_done, hi_heads)], axis=1)
            ob = ob + _dot(of, wob_v[pl.ds(2048 + hi_done * 128, (hi_heads - hi_done) * 128), :])
            hi_done = hi_heads
    assert hi_done == 16 and lo_done == 16 - NV // 2
    ob = ob + jnp.sum(acc8, axis=0, keepdims=True)

    res = gate * oa + (1.0 - gate) * ob
    out_ref[...] = res.astype(out_ref.dtype)


@jax.jit
def pallas_gated_mix__compressed_kv_cla__gqa_block_cached__decode_kernel(
    A_x, A_c_kv, A_w_q, A_w_uk, A_w_uv, A_w_o,
    B_x, B_k_cache, B_v_cache, B_wq, B_wo, gate_w,
):
    x = A_x.reshape(1, M)
    wqa = A_w_q.reshape(M * H, D)
    wuk = A_w_uk.reshape(C * H, D)
    wuv = A_w_uv.reshape(C * H, D)
    woa = A_w_o.reshape(H * D, M)
    ckv = A_c_kv.reshape(S, C)
    k = B_k_cache.reshape(H, S, D)
    v = B_v_cache.reshape(H, S, D)

    any_spec = pl.BlockSpec(memory_space=pl.ANY)
    out = pl.pallas_call(
        _kernel,
        in_specs=[any_spec] * 11,
        out_specs=pl.BlockSpec(memory_space=pltpu.VMEM),
        out_shape=jax.ShapeDtypeStruct((1, M), BF),
        scratch_shapes=[
            pltpu.VMEM((1, M), BF),
            pltpu.VMEM((M,), BF),
            pltpu.VMEM((M * H, D), BF),
            pltpu.VMEM((C * H, D), BF),
            pltpu.VMEM((S, C), BF),
            pltpu.VMEM((C * H, D), BF),
            pltpu.VMEM((H * D, M), BF),
            pltpu.VMEM((M, H * D), BF),
            pltpu.VMEM((H * D, M), BF),
            pltpu.VMEM((2, S, D), BF),
            pltpu.VMEM((2, S, D), BF),
            pltpu.VMEM((128, 4096), BF),
            pltpu.VMEM((H, 1, D), BF),
            pltpu.VMEM((H, 1, D), BF),
            pltpu.VMEM((1, S), F32),
            pltpu.VMEM((1, S), BF),
            pltpu.VMEM((1, D), F32),
            pltpu.VMEM((8, 4096), F32),
            pltpu.VMEM((128, 4096), BF),
            pltpu.VMEM((H, S), F32),
            pltpu.VMEM((H, C), F32),
            pltpu.VMEM((128, 4096), BF),
            pltpu.VMEM((1, 4096), F32),
            pltpu.SemaphoreType.DMA((NCH,)),
            pltpu.SemaphoreType.DMA((NCH,)),
            pltpu.SemaphoreType.DMA((WX + 5,)),
        ],
        compiler_params=pltpu.CompilerParams(
            vmem_limit_bytes=100 * 1024 * 1024,
            disable_bounds_checks=True,
            disable_semaphore_checks=True),
    )(x, gate_w, wqa, wuk, ckv, wuv, woa, B_wq, k, v, B_wo)
    return out.reshape(1, 1, M)
```

```python
import jax
import jax.numpy as jnp
import jax.experimental.pallas as pl
import jax.experimental.pallas.tpu as pltpu

H = 32
D = 128
S = 4096
M = 640
C = 512
BF = jnp.bfloat16
F32 = jnp.float32

CH = 256
NCH = S // CH
LO = 1
HI = 0
HW = 8
WX = 10
BUDGET = 100
SCALE = D ** -0.5

_NT = (((1,), (1,)), ((), ()))


def _dot(a, b):
    return jnp.dot(a, b, preferred_element_type=F32)


def _dot_nt(a, b):
    return jax.lax.dot_general(a, b, _NT, preferred_element_type=F32)


def _diag(n):
    r = jax.lax.broadcasted_iota(jnp.int32, (H, n), 0)
    c = jax.lax.broadcasted_iota(jnp.int32, (H, n), 1)
    return (c & 31) == r


def _kernel(x_hbm, gate_hbm, wqa_hbm, wuk_hbm, ckv_hbm, wuv_hbm, woa_hbm,
            wqb_hbm, k_hbm, v_hbm, wob_hbm,
            out_ref,
            x_v, gate_v, wqa_v, wuk_v, ckv_v, wuv_v, woa_v, wqb_v, wob_v,
            k_v, v_v, e_v, qb_v, ob_v, s_v, m_v, p0_v,
            xe_v, rt_v, sa_v, cc_v, ex_v, qacc_v,
            sem_k, sem_v, sem_h):
    lo_list, hi_list = [], []

    def add(lst, src, dst, rows):
        n = src.shape[0] // rows
        t0 = len(lst)
        for i in range(n):
            lst.append((src.at[pl.ds(i * rows, rows)], dst.at[pl.ds(i * rows, rows)]))
        return t0

    t_q = add(lo_list, wqa_hbm, wqa_v, 256)
    t_c = add(lo_list, ckv_hbm, ckv_v, 64)
    t_o = add(lo_list, woa_hbm, woa_v, 64)
    t_u = add(hi_list, wuk_hbm, wuk_v, 256)
    t_v = add(hi_list, wuv_hbm, wuv_v, 256)
    t_w = add(hi_list, wqb_hbm, wqb_v, 8)
    n_st = len(lo_list)
    assert n_st == len(hi_list) and n_st % NCH == 0

    def lo_copy(t):
        return pltpu.make_async_copy(lo_list[t][0], lo_list[t][1], sem_k.at[t % NCH])

    def hi_copy(t):
        return pltpu.make_async_copy(hi_list[t][0], hi_list[t][1], sem_v.at[t % NCH])

    def k_copy(h, slot, j):
        return pltpu.make_async_copy(k_hbm.at[h, pl.ds(j * CH, CH)], k_v.at[slot, pl.ds(j * CH, CH)],
                                     sem_k.at[j])

    def v_copy(h, slot, j):
        return pltpu.make_async_copy(v_hbm.at[h, pl.ds(j * CH, CH)], v_v.at[slot, pl.ds(j * CH, CH)],
                                     sem_v.at[j])

    def wol_copy(i):
        return pltpu.make_async_copy(wob_hbm.at[pl.ds(i * 64, 64)], wob_v.at[pl.ds(i * 64, 64)],
                                     sem_k.at[i % NCH])

    NH_SEM = WX + 5

    def woh_copy(i):
        return pltpu.make_async_copy(wob_hbm.at[pl.ds(2048 + i * 64, 64)], wob_v.at[pl.ds(2048 + i * 64, 64)],
                                     sem_h.at[i % NH_SEM])

    x_copy = pltpu.make_async_copy(x_hbm, x_v, sem_h.at[0])
    g_copy = pltpu.make_async_copy(gate_hbm, gate_v, sem_h.at[1])
    x_copy.start(priority=HI)
    g_copy.start(priority=HI)
    for t in range(NCH):
        lo_copy(t).start(priority=LO)
    for t in range(NCH):
        hi_copy(t).start(priority=HI)

    row = jax.lax.broadcasted_iota(jnp.int32, (128, 4096), 0)
    col = jax.lax.broadcasted_iota(jnp.int32, (128, 4096), 1)
    e_v[...] = jnp.where((col >> 5) == row, 1.0, 0.0).astype(BF)

    x_copy.wait()
    g_copy.wait()
    x = x_v[...]
    xf = x.astype(F32)
    gate = jax.nn.sigmoid(jnp.sum(xf * gate_v[...].astype(F32).reshape(1, M), axis=-1, keepdims=True))
    x5 = jnp.concatenate([x[:, b * 128:(b + 1) * 128] for b in range(5)]
                         + [jnp.zeros((3, 128), BF)], axis=0)
    xe = _dot(x5, e_v[...])
    xe_v[...] = xe

    st = {}

    QR = 256

    def q_item(i):
        def f():
            b, p = divmod(i, 4096 // QR)
            xr = xe_v[b:b + 1, QR * p:QR * (p + 1)]
            sb = jnp.where(_diag(QR), jnp.broadcast_to(xr, (H, QR)), 0.0).astype(BF)
            r = _dot(sb, wqa_v[pl.ds(QR * i, QR), :])
            st["qa"] = r if i == 0 else st["qa"] + r
            if i == 20480 // QR - 1:
                st["qa"] = st["qa"].astype(BF)
        return f

    def u_item(i):
        def f():
            b, p = divmod(i, 8)
            rt = _dot_nt(st["qa"], wuk_v[pl.ds(512 * i, 512), :])
            rt_v[32 * b:32 * (b + 1), 512 * p:512 * (p + 1)] = jnp.where(_diag(512), rt, 0.0).astype(BF)
        return f

    def gu_item(k):
        def f():
            r = _dot_nt(rt_v[:, 1024 * k:1024 * (k + 1)], e_v[:, 1024 * k:1024 * (k + 1)])
            st["qs"] = r if k == 0 else st["qs"] + r
            if k == 3:
                qs = st["qs"].astype(BF)
                st["qabs"] = jnp.concatenate([qs[32 * b:32 * (b + 1), :] for b in range(4)], axis=1)
        return f

    def c_item(i):
        def f():
            s = _dot_nt(st["qabs"], ckv_v[pl.ds(128 * i, 128), :])
            sa_v[:, 128 * i:128 * (i + 1)] = s
            st["mx"] = s if i == 0 else jnp.maximum(st["mx"], s)
            if i == 31:
                st["ma"] = jnp.max(st["mx"], axis=-1, keepdims=True)
        return f

    def pv_item(k):
        def f():
            p = jnp.exp((sa_v[:, 512 * k:512 * (k + 1)] - st["ma"]) * SCALE)
            ps = p[:, 0:128] + p[:, 128:256] + p[:, 256:384] + p[:, 384:512]
            st["ls"] = ps if k == 0 else st["ls"] + ps
            r = _dot(p.astype(BF), ckv_v[pl.ds(512 * k, 512), :])
            if k == 0:
                cc_v[...] = r
            elif k < 7:
                cc_v[...] = cc_v[...] + r
            else:
                la = jnp.sum(st["ls"], axis=-1, keepdims=True)
                cc = ((cc_v[...] + r) / la).astype(BF)
                st["cs"] = jnp.concatenate([cc[:, 128 * b:128 * (b + 1)] for b in range(4)], axis=0)
        return f

    def gv_item(k):
        def f():
            ex = _dot(st["cs"], e_v[:, 1024 * k:1024 * (k + 1)])
            r = jax.lax.broadcasted_iota(jnp.int32, (128, 1024), 0)
            c = jax.lax.broadcasted_iota(jnp.int32, (128, 1024), 1)
            ex_v[:, 1024 * k:1024 * (k + 1)] = jnp.where((c & 31) == (r & 31), ex, 0.0).astype(BF)
        return f

    def v_item(i):
        def f():
            b, p = divmod(i, 8)
            r = _dot(ex_v[32 * b:32 * (b + 1), 512 * p:512 * (p + 1)], wuv_v[pl.ds(512 * i, 512), :])
            st["ctx"] = r if i == 0 else st["ctx"] + r
            if i == 31:
                ctx = st["ctx"].astype(BF).astype(F32)
                st["cf"] = jnp.concatenate([ctx[h:h + 1, :] for h in range(H)], axis=1).astype(BF)
        return f

    def o_item(i):
        def f():
            r = _dot(st["cf"][:, 128 * i:128 * (i + 1)], woa_v[pl.ds(128 * i, 128), :])
            st["oa"] = r if i == 0 else st["oa"] + r
        return f

    def w_item(i):
        def f():
            b, p = divmod(i, 8)
            r = _dot(x[:, 128 * b:128 * (b + 1)], wqb_v[pl.ds(128 * b, 128), pl.ds(512 * p, 512)])
            if b == 0:
                qacc_v[:, 512 * p:512 * (p + 1)] = r
            elif b < 4:
                qacc_v[:, 512 * p:512 * (p + 1)] = qacc_v[:, 512 * p:512 * (p + 1)] + r
            else:
                qb = (qacc_v[:, 512 * p:512 * (p + 1)] + r).astype(BF)
                for hh in range(4):
                    qb_v[4 * p + hh] = qb[:, 128 * hh:128 * (hh + 1)]
        return f

    chain_a = []
    for i in range(20480 // QR):
        chain_a.append((t_q + (QR // 256) * (i + 1) - 1, 100 if QR == 256 else 32, q_item(i), i == 20480 // QR - 1))
    for i in range(32):
        chain_a.append((t_u + 2 * i + 1 - HW, 64, u_item(i), i in (25, 27, 29, 31)))
        if i in (25, 27, 29, 31):
            chain_a.append((0, 128, gu_item((i - 25) // 2), i == 31))
    for i in range(32):
        chain_a.append((t_c + 2 * i + 1, 64, c_item(i), i == 31))
    for k in range(8):
        chain_a.append((0, 128, pv_item(k), k == 7))
    for k in range(4):
        chain_a.append((0, 128, gv_item(k), True if k == 3 else False))
    for i in range(32):
        chain_a.append((t_v + 2 * i + 1 - HW, 32, v_item(i), i == 31))
    for i in range(32):
        chain_a.append((t_o + 2 * i + 1, 40, o_item(i), False))
    chain_w = [(t_w + 16 * (i // 8) + 15 - HW, 32, w_item(i), False) for i in range(40)]

    for t in range(HW):
        hi_copy(t).wait()
    ia = iw = 0
    for t in range(n_st):
        lo_copy(t).wait()
        if t + HW < n_st:
            hi_copy(t + HW).wait()
        if t + NCH < n_st:
            lo_copy(t + NCH).start(priority=LO)
            hi_copy(t + NCH).start(priority=HI)
        else:
            k_copy(0, 0, t + NCH - n_st).start(priority=LO)
        used = 0
        last = t == n_st - 1
        while ia < len(chain_a) and chain_a[ia][0] <= t and (used + chain_a[ia][1] <= BUDGET or used == 0 or last):
            used += chain_a[ia][1]
            chain_a[ia][2]()
            fence = chain_a[ia][3]
            ia += 1
            if fence and not last:
                break
        while iw < len(chain_w) and chain_w[iw][0] <= t and (used + chain_w[iw][1] <= BUDGET or used == 0 or last):
            used += chain_w[iw][1]
            chain_w[iw][2]()
            iw += 1
    assert ia == len(chain_a) and iw == len(chain_w)
    oa = st["oa"]

    def probs(j, m2):
        return jnp.exp((s_v[:, j * CH:(j + 1) * CH] - m2) * SCALE)

    def steps(h, do_pv, last):
        slot = h % 2
        pslot = 1 - slot
        q = qb_v[h]
        acc = jnp.zeros((1, D), F32)
        mx = None
        if do_pv:
            m2 = jnp.concatenate([m_v[...]] * (CH // D), axis=1)
            p = p0_v[...]
            lsum = jnp.zeros((1, D), F32)
        for j in range(NCH):
            k_copy(h, slot, j).wait()
            if do_pv:
                v_copy(h - 1, pslot, j).wait()
            if not last:
                k_copy(h + 1, pslot, j).start(priority=LO)
            else:
                wol_copy(j).start(priority=LO)
            v_copy(h, slot, j).start(priority=HI)
            sj = _dot_nt(q, k_v[slot, pl.ds(j * CH, CH), :])
            if do_pv:
                acc = acc + _dot(p.astype(BF), v_v[pslot, pl.ds(j * CH, CH), :])
                for c in range(CH // D):
                    lsum = lsum + p[:, c * D:(c + 1) * D]
                if j + 1 < NCH:
                    p = probs(j + 1, m2)
            s_v[:, j * CH:(j + 1) * CH] = sj
            for c in range(CH // D):
                sc = sj[:, c * D:(c + 1) * D]
                mx = sc if mx is None else jnp.maximum(mx, sc)
        m = jnp.broadcast_to(jnp.max(mx, axis=-1, keepdims=True), (1, D))
        m_v[...] = m
        p0_v[...] = probs(0, jnp.concatenate([m] * (CH // D), axis=1))
        if do_pv:
            ob_v[h - 1] = (acc / jnp.sum(lsum, axis=-1, keepdims=True)).astype(BF)

    steps(0, False, False)

    def head(h, carry):
        steps(h, True, False)
        return carry

    jax.lax.fori_loop(1, H - 1, head, 0)
    steps(H - 1, True, True)

    for i in range(WX):
        woh_copy(i).start(priority=HI)
    ob = jnp.zeros((1, M), F32)
    pslot = (H - 1) % 2
    NV = 2
    GRP = 4
    lo_done = 0
    hi_done = 0
    hi_waited = 0
    acc8 = None
    for i in range(H):
        wol_copy(i).wait()
        if i + NCH < H:
            wol_copy(i + NCH).start(priority=LO)
        if i + WX < H:
            woh_copy(i + WX).start(priority=HI)
        if i >= H - NV:
            r0 = 64 * i
            w = wob_v[pl.ds(r0, 64), :].astype(F32)
            oc = obc[r0 - 15 * 128:r0 - 15 * 128 + 64, :]
            pr = w * jnp.concatenate([oc] * 5, axis=1)
            pr = pr.reshape(8, 8, M).sum(axis=0)
            acc8 = pr if acc8 is None else acc8 + pr
            continue
        boundary = (i + 1) % GRP == 0 or i == H - NV - 1
        if not boundary:
            continue
        if i == GRP - 1:
            for j in range(NCH):
                v_copy(H - 1, pslot, j).wait()
            pl_ = jnp.exp((s_v[...] - m_v[:, 0:1]) * SCALE)
            ob_v[H - 1] = (_dot(pl_.astype(BF), v_v[pslot]) / jnp.sum(pl_, axis=-1, keepdims=True)).astype(BF)
            o15 = ob_v[15].astype(F32)
            obc = jnp.broadcast_to(o15, (128, 128)).T
        hi_avail = H if i == H - NV - 1 else min(H, i + 1 + 4)
        for ii in range(hi_waited, hi_avail):
            woh_copy(ii).wait()
        hi_waited = max(hi_waited, hi_avail)
        hi_heads = hi_waited // 2
        lo_heads = (i + 1) // 2
        if i == H - NV - 1 and NV < 2:
            raise NotImplementedError
        if lo_heads > lo_done:
            of = jnp.concatenate([ob_v[hh] for hh in range(lo_done, lo_heads)], axis=1)
            ob = ob + _dot(of, wob_v[pl.ds(lo_done * 128, (lo_heads - lo_done) * 128), :])
            lo_done = lo_heads
        if hi_heads > hi_done:
            of = jnp.concatenate([ob_v[16 + hh] for hh in range(hi_done, hi_heads)], axis=1)
            ob = ob + _dot(of, wob_v[pl.ds(2048 + hi_done * 128, (hi_heads - hi_done) * 128), :])
            hi_done = hi_heads
    assert hi_done == 16 and lo_done == 16 - NV // 2
    ob = ob + jnp.sum(acc8, axis=0, keepdims=True)

    res = gate * oa + (1.0 - gate) * ob
    out_ref[...] = res.astype(out_ref.dtype)


@jax.jit
def pallas_gated_mix__compressed_kv_cla__gqa_block_cached__decode_kernel(
    A_x, A_c_kv, A_w_q, A_w_uk, A_w_uv, A_w_o,
    B_x, B_k_cache, B_v_cache, B_wq, B_wo, gate_w,
):
    x = A_x.reshape(1, M)
    wqa = A_w_q.reshape(M * H, D)
    wuk = A_w_uk.reshape(C * H, D)
    wuv = A_w_uv.reshape(C * H, D)
    woa = A_w_o.reshape(H * D, M)
    ckv = A_c_kv.reshape(S, C)
    k = B_k_cache.reshape(H, S, D)
    v = B_v_cache.reshape(H, S, D)

    any_spec = pl.BlockSpec(memory_space=pl.ANY)
    out = pl.pallas_call(
        _kernel,
        in_specs=[any_spec] * 11,
        out_specs=pl.BlockSpec(memory_space=pltpu.VMEM),
        out_shape=jax.ShapeDtypeStruct((1, M), BF),
        scratch_shapes=[
            pltpu.VMEM((1, M), BF),
            pltpu.VMEM((M,), BF),
            pltpu.VMEM((M * H, D), BF),
            pltpu.VMEM((C * H, D), BF),
            pltpu.VMEM((S, C), BF),
            pltpu.VMEM((C * H, D), BF),
            pltpu.VMEM((H * D, M), BF),
            pltpu.VMEM((M, H * D), BF),
            pltpu.VMEM((H * D, M), BF),
            pltpu.VMEM((2, S, D), BF),
            pltpu.VMEM((2, S, D), BF),
            pltpu.VMEM((128, 4096), BF),
            pltpu.VMEM((H, 1, D), BF),
            pltpu.VMEM((H, 1, D), BF),
            pltpu.VMEM((1, S), F32),
            pltpu.VMEM((1, D), F32),
            pltpu.VMEM((1, CH), F32),
            pltpu.VMEM((8, 4096), F32),
            pltpu.VMEM((128, 4096), BF),
            pltpu.VMEM((H, S), F32),
            pltpu.VMEM((H, C), F32),
            pltpu.VMEM((128, 4096), BF),
            pltpu.VMEM((1, 4096), F32),
            pltpu.SemaphoreType.DMA((NCH,)),
            pltpu.SemaphoreType.DMA((NCH,)),
            pltpu.SemaphoreType.DMA((WX + 5,)),
        ],
        compiler_params=pltpu.CompilerParams(
            vmem_limit_bytes=100 * 1024 * 1024,
            disable_bounds_checks=True,
            disable_semaphore_checks=True),
    )(x, gate_w, wqa, wuk, ckv, wuv, woa, B_wq, k, v, B_wo)
    return out.reshape(1, 1, M)
```

```python
import jax
import jax.numpy as jnp
import jax.experimental.pallas as pl
import jax.experimental.pallas.tpu as pltpu

H = 32
D = 128
S = 4096
M = 640
C = 512
BF = jnp.bfloat16
F32 = jnp.float32

CH = 256
NCH = S // CH
LO = 1
HI = 0
HW = 8
WX = 10
BUDGET = 100
SCALE = D ** -0.5

_NT = (((1,), (1,)), ((), ()))


def _dot(a, b):
    return jnp.dot(a, b, preferred_element_type=F32)


def _dot_nt(a, b):
    return jax.lax.dot_general(a, b, _NT, preferred_element_type=F32)


def _diag(n):
    r = jax.lax.broadcasted_iota(jnp.int32, (H, n), 0)
    c = jax.lax.broadcasted_iota(jnp.int32, (H, n), 1)
    return (c & 31) == r


def _kernel(x_hbm, gate_hbm, wqa_hbm, wuk_hbm, ckv_hbm, wuv_hbm, woa_hbm,
            wqb_hbm, k_hbm, v_hbm, wob_hbm,
            out_ref,
            x_v, gate_v, wqa_v, wuk_v, ckv_v, wuv_v, woa_v, wqb_v, wob_v,
            k_v, v_v, e_v, qb_v, ob_v, s_v, m_v, p0_v,
            xe_v, rt_v, sa_v, cc_v, ex_v, qacc_v,
            sem_k, sem_v, sem_h):
    lo_list, hi_list = [], []

    def add(lst, src, dst, rows):
        n = src.shape[0] // rows
        t0 = len(lst)
        for i in range(n):
            lst.append((src.at[pl.ds(i * rows, rows)], dst.at[pl.ds(i * rows, rows)]))
        return t0

    t_q = add(lo_list, wqa_hbm, wqa_v, 256)
    t_c = add(lo_list, ckv_hbm, ckv_v, 64)
    t_o = add(lo_list, woa_hbm, woa_v, 64)
    halves = []
    for src, dst in ((wuk_hbm, wuk_v), (wuv_hbm, wuv_v)):
        halves += [(src, dst, i * 128, 128, None) for i in range(128)]
    halves += [(wqb_hbm, wqb_v, 8 * (i // 2), 8, 2048 * (i % 2)) for i in range(160)]
    HOFF = 1

    def descr(hs):
        out = []
        for src, dst, r0, n, c0 in hs:
            if out and c0 is None and out[-1][0] is src and out[-1][4] is None and out[-1][2] + out[-1][3] == r0:
                out[-1] = (src, dst, out[-1][2], out[-1][3] + n, None)
            else:
                out.append((src, dst, r0, n, c0))
        res = []
        for src, dst, r0, n, c0 in out:
            if c0 is None:
                res.append((src.at[pl.ds(r0, n)], dst.at[pl.ds(r0, n)]))
            else:
                res.append((src.at[pl.ds(r0, n), pl.ds(c0, 2048)], dst.at[pl.ds(r0, n), pl.ds(c0, 2048)]))
        return res

    hi_list = [descr(halves[2 * t + HOFF:2 * t + HOFF + 2]) for t in range(len(halves) // 2)]
    hi_first = descr(halves[:HOFF])
    t_u, t_v, t_w = 0, 64, 128
    n_st = len(lo_list)
    assert n_st == len(hi_list) and n_st % NCH == 0

    def lo_copy(t):
        return pltpu.make_async_copy(lo_list[t][0], lo_list[t][1], sem_k.at[t % NCH])

    class _Multi:
        def __init__(self, copies):
            self.copies = copies

        def start(self, priority):
            for c in self.copies:
                c.start(priority=priority)

        def wait(self):
            for c in self.copies:
                c.wait()

    def hi_copy(t):
        return _Multi([pltpu.make_async_copy(a, b, sem_v.at[t % NCH]) for a, b in hi_list[t]])

    def k_copy(h, slot, j):
        return pltpu.make_async_copy(k_hbm.at[h, pl.ds(j * CH, CH)], k_v.at[slot, pl.ds(j * CH, CH)],
                                     sem_k.at[j])

    VOFF = 128

    def v_rows(j):
        if VOFF == 0:
            return (j * CH, CH)
        if j == 0:
            return (0, VOFF)
        if j == NCH:
            return (S - CH + VOFF, CH - VOFF)
        return (j * CH - CH + VOFF, CH)

    def v_copy(h, slot, j):
        r0, n = v_rows(j)
        return pltpu.make_async_copy(v_hbm.at[h, pl.ds(r0, n)], v_v.at[slot, pl.ds(r0, n)], sem_v.at[j])

    NVP = NCH + (1 if VOFF else 0)

    def v_step_pieces(j):
        if VOFF == 0:
            return [j]
        return [j, NCH] if j == NCH - 1 else [j]

    v_issue_pieces = v_step_pieces

    def v_step_rows(j):
        r0 = v_rows(j)[0]
        return r0, sum(v_rows(pc)[1] for pc in v_step_pieces(j))

    def wol_copy(i):
        return pltpu.make_async_copy(wob_hbm.at[pl.ds(i * 64, 64)], wob_v.at[pl.ds(i * 64, 64)],
                                     sem_k.at[i % NCH])

    NH_SEM = WX + 5

    def woh_copy(i):
        return pltpu.make_async_copy(wob_hbm.at[pl.ds(2048 + i * 64, 64)], wob_v.at[pl.ds(2048 + i * 64, 64)],
                                     sem_h.at[i % NH_SEM])

    x_copy = pltpu.make_async_copy(x_hbm, x_v, sem_h.at[0])
    g_copy = pltpu.make_async_copy(gate_hbm, gate_v, sem_h.at[1])
    x_copy.start(priority=HI)
    g_copy.start(priority=HI)
    first_copy = _Multi([pltpu.make_async_copy(a, b, sem_h.at[2]) for a, b in hi_first])
    first_copy.start(priority=HI)
    for t in range(NCH):
        lo_copy(t).start(priority=LO)
    for t in range(NCH):
        hi_copy(t).start(priority=HI)

    row = jax.lax.broadcasted_iota(jnp.int32, (128, 4096), 0)
    col = jax.lax.broadcasted_iota(jnp.int32, (128, 4096), 1)
    e_v[...] = jnp.where((col >> 5) == row, 1.0, 0.0).astype(BF)

    x_copy.wait()
    g_copy.wait()
    first_copy.wait()
    x = x_v[...]
    xf = x.astype(F32)
    gate = jax.nn.sigmoid(jnp.sum(xf * gate_v[...].astype(F32).reshape(1, M), axis=-1, keepdims=True))
    x5 = jnp.concatenate([x[:, b * 128:(b + 1) * 128] for b in range(5)]
                         + [jnp.zeros((3, 128), BF)], axis=0)
    xe = _dot(x5, e_v[...])
    xe_v[...] = xe

    st = {}

    QR = 256

    def q_item(i):
        def f():
            b, p = divmod(i, 4096 // QR)
            xr = xe_v[b:b + 1, QR * p:QR * (p + 1)]
            sb = jnp.where(_diag(QR), jnp.broadcast_to(xr, (H, QR)), 0.0).astype(BF)
            r = _dot(sb, wqa_v[pl.ds(QR * i, QR), :])
            st["qa"] = r if i == 0 else st["qa"] + r
            if i == 20480 // QR - 1:
                st["qa"] = st["qa"].astype(BF)
        return f

    def u_item(i):
        def f():
            b, p = divmod(i, 8)
            rt = _dot_nt(st["qa"], wuk_v[pl.ds(512 * i, 512), :])
            rt_v[32 * b:32 * (b + 1), 512 * p:512 * (p + 1)] = jnp.where(_diag(512), rt, 0.0).astype(BF)
        return f

    def gu_item(k):
        def f():
            r = _dot_nt(rt_v[:, 1024 * k:1024 * (k + 1)], e_v[:, 1024 * k:1024 * (k + 1)])
            st["qs"] = r if k == 0 else st["qs"] + r
            if k == 3:
                qs = st["qs"].astype(BF)
                st["qabs"] = jnp.concatenate([qs[32 * b:32 * (b + 1), :] for b in range(4)], axis=1)
        return f

    def c_item(i):
        def f():
            s = _dot_nt(st["qabs"], ckv_v[pl.ds(128 * i, 128), :])
            sa_v[:, 128 * i:128 * (i + 1)] = s
            st["mx"] = s if i == 0 else jnp.maximum(st["mx"], s)
            if i == 31:
                st["ma"] = jnp.max(st["mx"], axis=-1, keepdims=True)
        return f

    def pv_item(k):
        def f():
            p = jnp.exp((sa_v[:, 512 * k:512 * (k + 1)] - st["ma"]) * SCALE)
            ps = p[:, 0:128] + p[:, 128:256] + p[:, 256:384] + p[:, 384:512]
            st["ls"] = ps if k == 0 else st["ls"] + ps
            r = _dot(p.astype(BF), ckv_v[pl.ds(512 * k, 512), :])
            if k == 0:
                cc_v[...] = r
            elif k < 7:
                cc_v[...] = cc_v[...] + r
            else:
                la = jnp.sum(st["ls"], axis=-1, keepdims=True)
                cc = ((cc_v[...] + r) / la).astype(BF)
                st["cs"] = jnp.concatenate([cc[:, 128 * b:128 * (b + 1)] for b in range(4)], axis=0)
        return f

    def gv_item(k):
        def f():
            ex = _dot(st["cs"], e_v[:, 1024 * k:1024 * (k + 1)])
            r = jax.lax.broadcasted_iota(jnp.int32, (128, 1024), 0)
            c = jax.lax.broadcasted_iota(jnp.int32, (128, 1024), 1)
            ex_v[:, 1024 * k:1024 * (k + 1)] = jnp.where((c & 31) == (r & 31), ex, 0.0).astype(BF)
        return f

    def v_item(i):
        def f():
            b, p = divmod(i, 8)
            r = _dot(ex_v[32 * b:32 * (b + 1), 512 * p:512 * (p + 1)], wuv_v[pl.ds(512 * i, 512), :])
            st["ctx"] = r if i == 0 else st["ctx"] + r
            if i == 31:
                ctx = st["ctx"].astype(BF).astype(F32)
                st["cf"] = jnp.concatenate([ctx[h:h + 1, :] for h in range(H)], axis=1).astype(BF)
        return f

    def o_item(i):
        def f():
            r = _dot(st["cf"][:, 128 * i:128 * (i + 1)], woa_v[pl.ds(128 * i, 128), :])
            st["oa"] = r if i == 0 else st["oa"] + r
        return f

    def w_item(i):
        def f():
            b, p = divmod(i, 8)
            r = _dot(x[:, 128 * b:128 * (b + 1)], wqb_v[pl.ds(128 * b, 128), pl.ds(512 * p, 512)])
            if b == 0:
                qacc_v[:, 512 * p:512 * (p + 1)] = r
            elif b < 4:
                qacc_v[:, 512 * p:512 * (p + 1)] = qacc_v[:, 512 * p:512 * (p + 1)] + r
            else:
                qb = (qacc_v[:, 512 * p:512 * (p + 1)] + r).astype(BF)
                for hh in range(4):
                    qb_v[4 * p + hh] = qb[:, 128 * hh:128 * (hh + 1)]
        return f

    chain_a = []
    for i in range(20480 // QR):
        chain_a.append((t_q + (QR // 256) * (i + 1) - 1, 100 if QR == 256 else 32, q_item(i), i == 20480 // QR - 1))
    for i in range(32):
        chain_a.append((t_u + 2 * i + 1 - HW, 64, u_item(i), i in (25, 27, 29, 31)))
        if i in (25, 27, 29, 31):
            chain_a.append((0, 128, gu_item((i - 25) // 2), i == 31))
    for i in range(32):
        chain_a.append((t_c + 2 * i + 1, 64, c_item(i), i == 31))
    for k in range(8):
        chain_a.append((0, 128, pv_item(k), k == 7))
    for k in range(4):
        chain_a.append((0, 128, gv_item(k), True if k == 3 else False))
    for i in range(32):
        chain_a.append((t_v + 2 * i + 1 - HW, 32, v_item(i), i == 31))
    for i in range(32):
        chain_a.append((t_o + 2 * i + 1, 40, o_item(i), False))
    chain_w = [(t_w + 16 * (i // 8) + 15 - HW, 32, w_item(i), False) for i in range(40)]

    for t in range(HW):
        hi_copy(t).wait()
    ia = iw = 0
    for t in range(n_st):
        lo_copy(t).wait()
        if t + HW < n_st:
            hi_copy(t + HW).wait()
        if t + NCH < n_st:
            lo_copy(t + NCH).start(priority=LO)
            hi_copy(t + NCH).start(priority=HI)
        else:
            k_copy(0, 0, t + NCH - n_st).start(priority=LO)
        used = 0
        last = t == n_st - 1
        while ia < len(chain_a) and chain_a[ia][0] <= t and (used + chain_a[ia][1] <= BUDGET or used == 0 or last):
            used += chain_a[ia][1]
            chain_a[ia][2]()
            fence = chain_a[ia][3]
            ia += 1
            if fence and not last:
                break
        while iw < len(chain_w) and chain_w[iw][0] <= t and (used + chain_w[iw][1] <= BUDGET or used == 0 or last):
            used += chain_w[iw][1]
            chain_w[iw][2]()
            iw += 1
    assert ia == len(chain_a) and iw == len(chain_w)
    oa = st["oa"]

    def probs(j, m):
        r0, n = v_step_rows(j)
        return jnp.exp((s_v[:, r0:r0 + n] - jnp.concatenate([m] * (n // D), axis=1)) * SCALE)

    def pv_dot(p, pslot, j):
        r0, n = v_step_rows(j)
        return _dot(p.astype(BF), v_v[pslot, pl.ds(r0, n), :])

    def steps(h, do_pv, last):
        slot = h % 2
        pslot = 1 - slot
        q = qb_v[h]
        acc = jnp.zeros((1, D), F32)
        mx = None
        if do_pv:
            m2 = m_v[...]
            p = p0_v[...]
            lsum = jnp.zeros((1, D), F32)
        for j in range(NCH):
            k_copy(h, slot, j).wait()
            if do_pv:
                for pc in v_step_pieces(j):
                    v_copy(h - 1, pslot, pc).wait()
            if not last:
                k_copy(h + 1, pslot, j).start(priority=LO)
            else:
                wol_copy(j).start(priority=LO)
            for pc in v_issue_pieces(j):
                v_copy(h, slot, pc).start(priority=HI)
            sj = _dot_nt(q, k_v[slot, pl.ds(j * CH, CH), :])
            if do_pv:
                acc = acc + pv_dot(p, pslot, j)
                for c in range(p.shape[1] // D):
                    lsum = lsum + p[:, c * D:(c + 1) * D]
                if j + 1 < NCH:
                    p = probs(j + 1, m2)
            s_v[:, j * CH:(j + 1) * CH] = sj
            for c in range(CH // D):
                sc = sj[:, c * D:(c + 1) * D]
                mx = sc if mx is None else jnp.maximum(mx, sc)
        m = jnp.broadcast_to(jnp.max(mx, axis=-1, keepdims=True), (1, D))
        m_v[...] = m
        p0_v[...] = probs(0, m)
        if do_pv:
            ob_v[h - 1] = (acc / jnp.sum(lsum, axis=-1, keepdims=True)).astype(BF)

    steps(0, False, False)

    def head(h, carry):
        steps(h, True, False)
        return carry

    jax.lax.fori_loop(1, H - 1, head, 0)
    steps(H - 1, True, True)

    for i in range(WX):
        woh_copy(i).start(priority=HI)
    ob = jnp.zeros((1, M), F32)
    pslot = (H - 1) % 2
    NV = 2
    GRP = 4
    lo_done = 0
    hi_done = 0
    hi_waited = 0
    acc8 = None
    for i in range(H):
        wol_copy(i).wait()
        if i + NCH < H:
            wol_copy(i + NCH).start(priority=LO)
        if i + WX < H:
            woh_copy(i + WX).start(priority=HI)
        if i >= H - NV:
            r0 = 64 * i
            w = wob_v[pl.ds(r0, 64), :].astype(F32)
            oc = obc[r0 - 15 * 128:r0 - 15 * 128 + 64, :]
            pr = w * jnp.concatenate([oc] * 5, axis=1)
            pr = pr.reshape(8, 8, M).sum(axis=0)
            acc8 = pr if acc8 is None else acc8 + pr
            continue
        boundary = (i + 1) % GRP == 0 or i == H - NV - 1
        if not boundary:
            continue
        if i == GRP - 1:
            for j in range(NVP):
                v_copy(H - 1, pslot, j).wait()
            pl_ = jnp.exp((s_v[...] - m_v[:, 0:1]) * SCALE)
            ob_v[H - 1] = (_dot(pl_.astype(BF), v_v[pslot]) / jnp.sum(pl_, axis=-1, keepdims=True)).astype(BF)
            o15 = ob_v[15].astype(F32)
            obc = jnp.broadcast_to(o15, (128, 128)).T
        hi_avail = H if i == H - NV - 1 else min(H, i + 1 + 4)
        for ii in range(hi_waited, hi_avail):
            woh_copy(ii).wait()
        hi_waited = max(hi_waited, hi_avail)
        hi_heads = hi_waited // 2
        lo_heads = (i + 1) // 2
        if i == H - NV - 1 and NV < 2:
            raise NotImplementedError
        if lo_heads > lo_done:
            of = jnp.concatenate([ob_v[hh] for hh in range(lo_done, lo_heads)], axis=1)
            ob = ob + _dot(of, wob_v[pl.ds(lo_done * 128, (lo_heads - lo_done) * 128), :])
            lo_done = lo_heads
        if hi_heads > hi_done:
            of = jnp.concatenate([ob_v[16 + hh] for hh in range(hi_done, hi_heads)], axis=1)
            ob = ob + _dot(of, wob_v[pl.ds(2048 + hi_done * 128, (hi_heads - hi_done) * 128), :])
            hi_done = hi_heads
    assert hi_done == 16 and lo_done == 16 - NV // 2
    ob = ob + jnp.sum(acc8, axis=0, keepdims=True)

    res = gate * oa + (1.0 - gate) * ob
    out_ref[...] = res.astype(out_ref.dtype)


@jax.jit
def pallas_gated_mix__compressed_kv_cla__gqa_block_cached__decode_kernel(
    A_x, A_c_kv, A_w_q, A_w_uk, A_w_uv, A_w_o,
    B_x, B_k_cache, B_v_cache, B_wq, B_wo, gate_w,
):
    x = A_x.reshape(1, M)
    wqa = A_w_q.reshape(M * H, D)
    wuk = A_w_uk.reshape(C * H, D)
    wuv = A_w_uv.reshape(C * H, D)
    woa = A_w_o.reshape(H * D, M)
    ckv = A_c_kv.reshape(S, C)
    k = B_k_cache.reshape(H, S, D)
    v = B_v_cache.reshape(H, S, D)

    any_spec = pl.BlockSpec(memory_space=pl.ANY)
    out = pl.pallas_call(
        _kernel,
        in_specs=[any_spec] * 11,
        out_specs=pl.BlockSpec(memory_space=pltpu.VMEM),
        out_shape=jax.ShapeDtypeStruct((1, M), BF),
        scratch_shapes=[
            pltpu.VMEM((1, M), BF),
            pltpu.VMEM((M,), BF),
            pltpu.VMEM((M * H, D), BF),
            pltpu.VMEM((C * H, D), BF),
            pltpu.VMEM((S, C), BF),
            pltpu.VMEM((C * H, D), BF),
            pltpu.VMEM((H * D, M), BF),
            pltpu.VMEM((M, H * D), BF),
            pltpu.VMEM((H * D, M), BF),
            pltpu.VMEM((2, S, D), BF),
            pltpu.VMEM((2, S, D), BF),
            pltpu.VMEM((128, 4096), BF),
            pltpu.VMEM((H, 1, D), BF),
            pltpu.VMEM((H, 1, D), BF),
            pltpu.VMEM((1, S), F32),
            pltpu.VMEM((1, D), F32),
            pltpu.VMEM((1, 128), F32),
            pltpu.VMEM((8, 4096), F32),
            pltpu.VMEM((128, 4096), BF),
            pltpu.VMEM((H, S), F32),
            pltpu.VMEM((H, C), F32),
            pltpu.VMEM((128, 4096), BF),
            pltpu.VMEM((1, 4096), F32),
            pltpu.SemaphoreType.DMA((NCH,)),
            pltpu.SemaphoreType.DMA((NCH + 1,)),
            pltpu.SemaphoreType.DMA((WX + 5,)),
        ],
        compiler_params=pltpu.CompilerParams(
            vmem_limit_bytes=100 * 1024 * 1024,
            disable_bounds_checks=True,
            disable_semaphore_checks=True),
    )(x, gate_w, wqa, wuk, ckv, wuv, woa, B_wq, k, v, B_wo)
    return out.reshape(1, 1, M)
```

```python
import jax
import jax.numpy as jnp
import jax.experimental.pallas as pl
import jax.experimental.pallas.tpu as pltpu

H = 32
D = 128
S = 4096
M = 640
C = 512
BF = jnp.bfloat16
F32 = jnp.float32
SCALE = D ** -0.5

CH = 256
NCH = S // CH
VOFF = 128
LO = 1
HI = 0
HW = 8
BUDGET = 100
WX = 10
WA = 4
GRP = 4
NV = 2
NH_SEM = WX + 5

_NT = (((1,), (1,)), ((), ()))


def _dot(a, b):
    return jnp.dot(a, b, preferred_element_type=F32)


def _dot_nt(a, b):
    return jax.lax.dot_general(a, b, _NT, preferred_element_type=F32)


def _diag(rows, cols):
    r = jax.lax.broadcasted_iota(jnp.int32, (rows, cols), 0)
    c = jax.lax.broadcasted_iota(jnp.int32, (rows, cols), 1)
    return (c & 31) == (r & 31)


class _Copies:
    def __init__(self, pairs, sem):
        self.copies = [pltpu.make_async_copy(src, dst, sem) for src, dst in pairs]

    def start(self, priority):
        for c in self.copies:
            c.start(priority=priority)

    def wait(self):
        for c in self.copies:
            c.wait()


def _kernel(x_hbm, gate_hbm, wqa_hbm, wuk_hbm, ckv_hbm, wuv_hbm, woa_hbm,
            wqb_hbm, k_hbm, v_hbm, wob_hbm,
            out_ref,
            x_v, gate_v, wqa_v, wuk_v, ckv_v, wuv_v, woa_v, wqb_v, wob_v,
            k_v, v_v, e_v, qb_v, ob_v, s_v, m_v, p0_v,
            xe_v, rt_v, sa_v, cc_v, ex_v, qacc_v,
            sem_lo, sem_hi, sem_x):
    lo_list = []

    def add_lo(src, dst, rows):
        t0 = len(lo_list)
        for i in range(src.shape[0] // rows):
            lo_list.append((src.at[pl.ds(i * rows, rows)], dst.at[pl.ds(i * rows, rows)]))
        return t0

    t_q = add_lo(wqa_hbm, wqa_v, 256)
    t_c = add_lo(ckv_hbm, ckv_v, 64)
    t_o = add_lo(woa_hbm, woa_v, 64)
    n_st = len(lo_list)

    halves = []
    for src, dst in ((wuk_hbm, wuk_v), (wuv_hbm, wuv_v)):
        halves += [(src, dst, i * 128, 128, None) for i in range(128)]
    halves += [(wqb_hbm, wqb_v, 8 * (i // 2), 8, 2048 * (i % 2)) for i in range(160)]

    def slices(hs):
        merged = []
        for src, dst, r0, n, c0 in hs:
            if merged and c0 is None and merged[-1][0] is src and merged[-1][2] + merged[-1][3] == r0:
                merged[-1] = (src, dst, merged[-1][2], merged[-1][3] + n, None)
            else:
                merged.append((src, dst, r0, n, c0))
        out = []
        for src, dst, r0, n, c0 in merged:
            if c0 is None:
                out.append((src.at[pl.ds(r0, n)], dst.at[pl.ds(r0, n)]))
            else:
                out.append((src.at[pl.ds(r0, n), pl.ds(c0, 2048)], dst.at[pl.ds(r0, n), pl.ds(c0, 2048)]))
        return out

    hi_list = [slices(halves[2 * t + 1:2 * t + 3]) for t in range(len(halves) // 2)]
    t_u, t_v, t_w = 0, 64, 128
    assert n_st == len(hi_list) and n_st % NCH == 0

    def lo_copy(t):
        return pltpu.make_async_copy(lo_list[t][0], lo_list[t][1], sem_lo.at[t % NCH])

    def hi_copy(t):
        return _Copies(hi_list[t], sem_hi.at[t % NCH])

    def k_copy(h, slot, j):
        return pltpu.make_async_copy(k_hbm.at[h, pl.ds(j * CH, CH)], k_v.at[slot, pl.ds(j * CH, CH)],
                                     sem_lo.at[j])

    def v_rows(pc):
        if pc == 0:
            return 0, VOFF
        if pc == NCH:
            return S - CH + VOFF, CH - VOFF
        return pc * CH - CH + VOFF, CH

    def v_pieces(j):
        return [j, NCH] if j == NCH - 1 else [j]

    def v_step_rows(j):
        return v_rows(j)[0], sum(v_rows(pc)[1] for pc in v_pieces(j))

    def v_copy(h, slot, pc):
        r0, n = v_rows(pc)
        return pltpu.make_async_copy(v_hbm.at[h, pl.ds(r0, n)], v_v.at[slot, pl.ds(r0, n)], sem_hi.at[pc])

    def wol_copy(i):
        return pltpu.make_async_copy(wob_hbm.at[pl.ds(i * 64, 64)], wob_v.at[pl.ds(i * 64, 64)],
                                     sem_lo.at[i % NCH])

    def woh_copy(i):
        return pltpu.make_async_copy(wob_hbm.at[pl.ds(2048 + i * 64, 64)], wob_v.at[pl.ds(2048 + i * 64, 64)],
                                     sem_x.at[i % NH_SEM])

    x_copy = pltpu.make_async_copy(x_hbm, x_v, sem_x.at[0])
    g_copy = pltpu.make_async_copy(gate_hbm, gate_v, sem_x.at[1])
    first_copy = _Copies(slices(halves[:1]), sem_x.at[2])
    x_copy.start(priority=HI)
    g_copy.start(priority=HI)
    first_copy.start(priority=HI)
    for t in range(NCH):
        lo_copy(t).start(priority=LO)
    for t in range(NCH):
        hi_copy(t).start(priority=HI)

    row = jax.lax.broadcasted_iota(jnp.int32, (128, 4096), 0)
    col = jax.lax.broadcasted_iota(jnp.int32, (128, 4096), 1)
    e_v[...] = jnp.where((col >> 5) == row, 1.0, 0.0).astype(BF)

    x_copy.wait()
    g_copy.wait()
    first_copy.wait()
    x = x_v[...]
    gate = jax.nn.sigmoid(jnp.sum(x.astype(F32) * gate_v[...].astype(F32).reshape(1, M), axis=-1, keepdims=True))
    x5 = jnp.concatenate([x[:, b * 128:(b + 1) * 128] for b in range(5)]
                         + [jnp.zeros((3, 128), BF)], axis=0)
    xe_v[...] = _dot(x5, e_v[...])

    st = {}

    def q_item(i):
        def f():
            b, p = divmod(i, 16)
            xr = xe_v[b:b + 1, 256 * p:256 * (p + 1)]
            sb = jnp.where(_diag(H, 256), jnp.broadcast_to(xr, (H, 256)), 0.0).astype(BF)
            r = _dot(sb, wqa_v[pl.ds(256 * i, 256), :])
            st["qa"] = r if i == 0 else st["qa"] + r
            if i == 79:
                st["qa"] = st["qa"].astype(BF)
        return f

    def u_item(i):
        def f():
            b, p = divmod(i, 8)
            rt = _dot_nt(st["qa"], wuk_v[pl.ds(512 * i, 512), :])
            rt_v[32 * b:32 * (b + 1), 512 * p:512 * (p + 1)] = jnp.where(_diag(H, 512), rt, 0.0).astype(BF)
        return f

    def gu_item(k):
        def f():
            r = _dot_nt(rt_v[:, 1024 * k:1024 * (k + 1)], e_v[:, 1024 * k:1024 * (k + 1)])
            st["qs"] = r if k == 0 else st["qs"] + r
            if k == 3:
                qs = st["qs"].astype(BF)
                st["qabs"] = jnp.concatenate([qs[32 * b:32 * (b + 1), :] for b in range(4)], axis=1)
        return f

    def c_item(i):
        def f():
            s = _dot_nt(st["qabs"], ckv_v[pl.ds(128 * i, 128), :])
            sa_v[:, 128 * i:128 * (i + 1)] = s
            st["mx"] = s if i == 0 else jnp.maximum(st["mx"], s)
            if i == 31:
                st["ma"] = jnp.max(st["mx"], axis=-1, keepdims=True)
        return f

    def pv_item(k):
        def f():
            p = jnp.exp((sa_v[:, 512 * k:512 * (k + 1)] - st["ma"]) * SCALE)
            ps = p[:, 0:128] + p[:, 128:256] + p[:, 256:384] + p[:, 384:512]
            st["ls"] = ps if k == 0 else st["ls"] + ps
            r = _dot(p.astype(BF), ckv_v[pl.ds(512 * k, 512), :])
            if k == 0:
                cc_v[...] = r
            elif k < 7:
                cc_v[...] = cc_v[...] + r
            else:
                la = jnp.sum(st["ls"], axis=-1, keepdims=True)
                cc = ((cc_v[...] + r) / la).astype(BF)
                st["cs"] = jnp.concatenate([cc[:, 128 * b:128 * (b + 1)] for b in range(4)], axis=0)
        return f

    def gv_item(k):
        def f():
            ex = _dot(st["cs"], e_v[:, 1024 * k:1024 * (k + 1)])
            ex_v[:, 1024 * k:1024 * (k + 1)] = jnp.where(_diag(128, 1024), ex, 0.0).astype(BF)
        return f

    def v_item(i):
        def f():
            b, p = divmod(i, 8)
            r = _dot(ex_v[32 * b:32 * (b + 1), 512 * p:512 * (p + 1)], wuv_v[pl.ds(512 * i, 512), :])
            st["ctx"] = r if i == 0 else st["ctx"] + r
            if i == 31:
                ctx = st["ctx"].astype(BF).astype(F32)
                st["cf"] = jnp.concatenate([ctx[h:h + 1, :] for h in range(H)], axis=1).astype(BF)
        return f

    def o_item(i):
        def f():
            r = _dot(st["cf"][:, 128 * i:128 * (i + 1)], woa_v[pl.ds(128 * i, 128), :])
            st["oa"] = r if i == 0 else st["oa"] + r
        return f

    def w_item(i):
        def f():
            b, p = divmod(i, 8)
            r = _dot(x[:, 128 * b:128 * (b + 1)], wqb_v[pl.ds(128 * b, 128), pl.ds(512 * p, 512)])
            if b == 0:
                qacc_v[:, 512 * p:512 * (p + 1)] = r
            elif b < 4:
                qacc_v[:, 512 * p:512 * (p + 1)] = qacc_v[:, 512 * p:512 * (p + 1)] + r
            else:
                qb = (qacc_v[:, 512 * p:512 * (p + 1)] + r).astype(BF)
                for hh in range(4):
                    qb_v[4 * p + hh] = qb[:, 128 * hh:128 * (hh + 1)]
        return f

    chain_a = []
    for i in range(80):
        chain_a.append((t_q + i, BUDGET, q_item(i), i == 79))
    for i in range(32):
        chain_a.append((t_u + 2 * i + 1 - HW, 64, u_item(i), i in (25, 27, 29, 31)))
        if i in (25, 27, 29, 31):
            chain_a.append((0, 128, gu_item((i - 25) // 2), i == 31))
    for i in range(32):
        chain_a.append((t_c + 2 * i + 1, 64, c_item(i), i == 31))
    for k in range(8):
        chain_a.append((0, 128, pv_item(k), k == 7))
    for k in range(4):
        chain_a.append((0, 128, gv_item(k), k == 3))
    for i in range(32):
        chain_a.append((t_v + 2 * i + 1 - HW, 32, v_item(i), i == 31))
    for i in range(32):
        chain_a.append((t_o + 2 * i + 1, 40, o_item(i), False))
    chain_w = [(t_w + 16 * (i // 8) + 15 - HW, 32, w_item(i), False) for i in range(40)]

    for t in range(HW):
        hi_copy(t).wait()
    ia = iw = 0
    for t in range(n_st):
        lo_copy(t).wait()
        if t + HW < n_st:
            hi_copy(t + HW).wait()
        if t + NCH < n_st:
            lo_copy(t + NCH).start(priority=LO)
            hi_copy(t + NCH).start(priority=HI)
        else:
            k_copy(0, 0, t + NCH - n_st).start(priority=LO)
        used = 0
        last = t == n_st - 1
        while ia < len(chain_a) and chain_a[ia][0] <= t and (used + chain_a[ia][1] <= BUDGET or used == 0 or last):
            used += chain_a[ia][1]
            chain_a[ia][2]()
            fence = chain_a[ia][3]
            ia += 1
            if fence and not last:
                break
        while iw < len(chain_w) and chain_w[iw][0] <= t and (used + chain_w[iw][1] <= BUDGET or used == 0 or last):
            used += chain_w[iw][1]
            chain_w[iw][2]()
            iw += 1
    assert ia == len(chain_a) and iw == len(chain_w)
    oa = st["oa"]

    def probs(j, m):
        r0, n = v_step_rows(j)
        return jnp.exp((s_v[:, r0:r0 + n] - jnp.concatenate([m] * (n // D), axis=1)) * SCALE)

    def steps(h, do_pv, last):
        slot = h % 2
        pslot = 1 - slot
        q = qb_v[h]
        acc = jnp.zeros((1, D), F32)
        mx = None
        if do_pv:
            m_prev = m_v[...]
            p = p0_v[...]
            lsum = jnp.zeros((1, D), F32)
        for j in range(NCH):
            k_copy(h, slot, j).wait()
            if do_pv:
                for pc in v_pieces(j):
                    v_copy(h - 1, pslot, pc).wait()
            if not last:
                k_copy(h + 1, pslot, j).start(priority=LO)
            else:
                wol_copy(j).start(priority=LO)
            for pc in v_pieces(j):
                v_copy(h, slot, pc).start(priority=HI)
            sj = _dot_nt(q, k_v[slot, pl.ds(j * CH, CH), :])
            if do_pv:
                r0, n = v_step_rows(j)
                acc = acc + _dot(p.astype(BF), v_v[pslot, pl.ds(r0, n), :])
                for c in range(n // D):
                    lsum = lsum + p[:, c * D:(c + 1) * D]
                if j + 1 < NCH:
                    p = probs(j + 1, m_prev)
            s_v[:, j * CH:(j + 1) * CH] = sj
            for c in range(CH // D):
                sc = sj[:, c * D:(c + 1) * D]
                mx = sc if mx is None else jnp.maximum(mx, sc)
        m = jnp.broadcast_to(jnp.max(mx, axis=-1, keepdims=True), (1, D))
        m_v[...] = m
        p0_v[...] = probs(0, m)
        if do_pv:
            ob_v[h - 1] = (acc / jnp.sum(lsum, axis=-1, keepdims=True)).astype(BF)

    steps(0, False, False)

    def head(h, carry):
        steps(h, True, False)
        return carry

    jax.lax.fori_loop(1, H - 1, head, 0)
    steps(H - 1, True, True)

    for i in range(WX):
        woh_copy(i).start(priority=HI)
    ob = jnp.zeros((1, M), F32)
    pslot = (H - 1) % 2
    lo_done = hi_done = hi_waited = 0
    acc8 = None
    obc = None
    for i in range(H):
        wol_copy(i).wait()
        if i + NCH < H:
            wol_copy(i + NCH).start(priority=LO)
        if i + WX < H:
            woh_copy(i + WX).start(priority=HI)
        if i >= H - NV:
            r0 = 64 * i
            w = wob_v[pl.ds(r0, 64), :].astype(F32)
            oc = obc[r0 - 15 * 128:r0 - 15 * 128 + 64, :]
            pr = (w * jnp.concatenate([oc] * 5, axis=1)).reshape(8, 8, M).sum(axis=0)
            acc8 = pr if acc8 is None else acc8 + pr
            continue
        if (i + 1) % GRP != 0 and i != H - NV - 1:
            continue
        if i == GRP - 1:
            for pc in range(NCH + 1):
                v_copy(H - 1, pslot, pc).wait()
            pl_ = jnp.exp((s_v[...] - m_v[:, 0:1]) * SCALE)
            ob_v[H - 1] = (_dot(pl_.astype(BF), v_v[pslot]) / jnp.sum(pl_, axis=-1, keepdims=True)).astype(BF)
            obc = jnp.broadcast_to(ob_v[15].astype(F32), (128, 128)).T
        hi_avail = H if i == H - NV - 1 else min(H, i + 1 + WA)
        for ii in range(hi_waited, hi_avail):
            woh_copy(ii).wait()
        hi_waited = hi_avail
        lo_heads, hi_heads = (i + 1) // 2, hi_waited // 2
        if lo_heads > lo_done:
            of = jnp.concatenate([ob_v[hh] for hh in range(lo_done, lo_heads)], axis=1)
            ob = ob + _dot(of, wob_v[pl.ds(lo_done * 128, (lo_heads - lo_done) * 128), :])
            lo_done = lo_heads
        if hi_heads > hi_done:
            of = jnp.concatenate([ob_v[16 + hh] for hh in range(hi_done, hi_heads)], axis=1)
            ob = ob + _dot(of, wob_v[pl.ds(2048 + hi_done * 128, (hi_heads - hi_done) * 128), :])
            hi_done = hi_heads
    assert hi_done == 16 and lo_done == 16 - NV // 2
    ob = ob + jnp.sum(acc8, axis=0, keepdims=True)

    out_ref[...] = (gate * oa + (1.0 - gate) * ob).astype(out_ref.dtype)


@jax.jit
def pallas_gated_mix__compressed_kv_cla__gqa_block_cached__decode_kernel(
    A_x, A_c_kv, A_w_q, A_w_uk, A_w_uv, A_w_o,
    B_x, B_k_cache, B_v_cache, B_wq, B_wo, gate_w,
):
    del B_x
    x = A_x.reshape(1, M)
    wqa = A_w_q.reshape(M * H, D)
    wuk = A_w_uk.reshape(C * H, D)
    wuv = A_w_uv.reshape(C * H, D)
    woa = A_w_o.reshape(H * D, M)
    ckv = A_c_kv.reshape(S, C)
    k = B_k_cache.reshape(H, S, D)
    v = B_v_cache.reshape(H, S, D)

    any_spec = pl.BlockSpec(memory_space=pl.ANY)
    out = pl.pallas_call(
        _kernel,
        in_specs=[any_spec] * 11,
        out_specs=pl.BlockSpec(memory_space=pltpu.VMEM),
        out_shape=jax.ShapeDtypeStruct((1, M), BF),
        scratch_shapes=[
            pltpu.VMEM((1, M), BF),
            pltpu.VMEM((M,), BF),
            pltpu.VMEM((M * H, D), BF),
            pltpu.VMEM((C * H, D), BF),
            pltpu.VMEM((S, C), BF),
            pltpu.VMEM((C * H, D), BF),
            pltpu.VMEM((H * D, M), BF),
            pltpu.VMEM((M, H * D), BF),
            pltpu.VMEM((H * D, M), BF),
            pltpu.VMEM((2, S, D), BF),
            pltpu.VMEM((2, S, D), BF),
            pltpu.VMEM((128, 4096), BF),
            pltpu.VMEM((H, 1, D), BF),
            pltpu.VMEM((H, 1, D), BF),
            pltpu.VMEM((1, S), F32),
            pltpu.VMEM((1, D), F32),
            pltpu.VMEM((1, VOFF), F32),
            pltpu.VMEM((8, 4096), F32),
            pltpu.VMEM((128, 4096), BF),
            pltpu.VMEM((H, S), F32),
            pltpu.VMEM((H, C), F32),
            pltpu.VMEM((128, 4096), BF),
            pltpu.VMEM((1, 4096), F32),
            pltpu.SemaphoreType.DMA((NCH,)),
            pltpu.SemaphoreType.DMA((NCH + 1,)),
            pltpu.SemaphoreType.DMA((NH_SEM,)),
        ],
        compiler_params=pltpu.CompilerParams(
            vmem_limit_bytes=100 * 1024 * 1024,
            disable_semaphore_checks=True),
    )(x, gate_w, wqa, wuk, ckv, wuv, woa, B_wq, k, v, B_wo)
    return out.reshape(1, 1, M)
```
